```python
import os as _os
_os.environ.setdefault('JAX_PLATFORMS', 'cpu')
import jax
import jax.numpy as jnp

def _softmax(x, axis=-1):
    return jax.nn.softmax(x, axis=axis)

def _gelu(x):
    return jax.nn.gelu(x, approximate=True)

def _silu(x):
    return jax.nn.silu(x)

def _sigmoid(x):
    return jax.nn.sigmoid(x)

def _layernorm(x, axis=-1, eps=1e-05):
    m = jnp.mean(x, axis=axis, keepdims=True)
    v = jnp.var(x, axis=axis, keepdims=True)
    return (x - m) / jnp.sqrt(v + eps)

def _scatter_add(tgt, idx, src, axis=0):
    return tgt.at[idx].add(src)

def _segment_sum(src, seg, n):
    return jax.ops.segment_sum(src, seg, n)

class _Rng:

    def __init__(self, key):
        self._k = key

    def _next(self):
        self._k, sub = jax.random.split(self._k)
        return sub

    def normal(self, shape):
        return jax.random.normal(self._next(), shape, dtype=jnp.bfloat16)

    def randint(self, lo, hi, shape):
        return jax.random.randint(self._next(), shape, lo, hi, dtype=jnp.int32)

    def uniform(self, shape, lo=0.0, hi=1.0):
        return jax.random.uniform(self._next(), shape, jnp.bfloat16, lo, hi)

    def permutation(self, n):
        return jax.random.permutation(self._next(), n)
kernel_name = 'adaLN_cond__softmax_full_mha__mixer_gmlp__prompt'

def setup_inputs():
    _rng = _Rng(jax.random.key(int.from_bytes(__import__("os").urandom(4), "little")))
    _w = lambda a: (lambda t: t.astype(jnp.bfloat16) if jnp.issubdtype(t.dtype, jnp.floating) else t)(jnp.asarray(a))

    def _A_setup():
        B, S, D = (1, 2048, 512)
        return {'x': _w((lambda *s: _rng.normal(s) * 0.05)(B, S, D)), 'wqkv': _w((lambda *s: _rng.normal(s) * 0.05)(D, 3 * D)), 'wo': _w((lambda *s: _rng.normal(s) * 0.05)(D, D))}
    _A_in = _A_setup()

    def _B_setup():
        B, S, D, F = (1, 2048, 512, 1792)
        Fh = F // 2
        return {'x': _w((lambda *s: _rng.normal(s) * 0.05)(B, S, D)), 'w_in': _w((lambda *s: _rng.normal(s) * 0.4)(D, 2 * Fh)), 'w_sp': _w(0.01 * (lambda *s: _rng.normal(s) * 0.4)(S, S)), 'b_sp': _w(1.0 + 0.01 * (lambda *s: _rng.normal(s) * 0.05)(S)), 'w_out': _w((lambda *s: _rng.normal(s) * 0.05)(Fh, D))}
    _B_in = _B_setup()
    return {'A_x': _A_in['x'], 'A_wqkv': _A_in['wqkv'], 'A_wo': _A_in['wo'], 'B_x': _B_in['x'], 'B_w_in': _B_in['w_in'], 'B_w_sp': _B_in['w_sp'], 'B_b_sp': _B_in['b_sp'], 'B_w_out': _B_in['w_out'], 'c': _w((lambda *s: _rng.normal(s) * 0.05)(1, 512) * 8.0), 'w_mod': _w((lambda *s: _rng.normal(s) * 0.05)(512, 6 * 512) * 512 ** (-0.5) * 8.0)}

def reference(A_x, A_wqkv, A_wo, B_x, B_w_in, B_w_sp, B_b_sp, B_w_out, c, w_mod):

    def _A_ref(x, wqkv, wo):
        B, S, D = x.shape
        H = 32
        Dh = D // H
        qkv = (lambda x, *d: x.transpose(*d))((x @ wqkv).reshape(B, S, 3, H, Dh), 2, 0, 3, 1, 4)
        q, k, v = (qkv[0], qkv[1], qkv[2])
        scale = Dh ** (-0.5)
        scores = jnp.einsum('bhqd,bhkd->bhqk', q, k) * scale
        p = _softmax(scores, axis=-1)
        o = jnp.einsum('bhqk,bhkd->bhqd', p, v)
        return (lambda x, *d: x.transpose(*d))(o, 0, 2, 1, 3).reshape(B, S, D) @ wo

    def _B_ref(x, w_in, w_sp, b_sp, w_out):
        B, S, D = x.shape
        F = w_in.shape[-1]
        Fh = F // 2
        z = _gelu(jnp.einsum('bsd,df->bsf', x, w_in))
        z1 = z[..., :Fh].copy()
        z2 = _layernorm(z[..., Fh:], axis=-1)
        g = jnp.einsum('ts,bsf->btf', w_sp, z2) + b_sp[None, :, None]
        return jnp.einsum('bsf,fd->bsd', z1 * g, w_out)
    x = A_x
    mod = (_silu(c) @ w_mod).reshape(c.shape[0], 6, 1, -1)
    sa, ca, ga, sb, cb, gb = (mod[:, 0].copy(), mod[:, 1].copy(), mod[:, 2].copy(), mod[:, 3].copy(), mod[:, 4].copy(), mod[:, 5].copy())
    h = _layernorm(x, axis=-1) * (1 + ca) + sa
    x = x + ga * _A_ref(h, A_wqkv, A_wo)
    h = _layernorm(x, axis=-1) * (1 + cb) + sb
    x = x + gb * _B_ref(h, B_w_in, B_w_sp, B_b_sp, B_w_out)
    return x
```

```python
import math

import jax
import jax.numpy as jnp
from jax import lax
import jax.experimental.pallas as pl
import jax.experimental.pallas.tpu as pltpu

S = 2048
D = 512
H = 32
DH = 16
FH = 896
EPS = 1e-5

TQ = 512
NJ = S // TQ
CK = 128
NC = S // CK
UN = 8
SKEW = 2
TP = 512
TM1 = 256
TM2 = 256

L_LO = 2.0 ** -60
L_HI = 2.0 ** 60

F32 = jnp.float32
BF16 = jnp.bfloat16
U32 = jnp.uint32


def _ln(x):
    m = jnp.mean(x, axis=-1, keepdims=True)
    xc = x - m
    v = jnp.mean(xc * xc, axis=-1, keepdims=True)
    return xc * lax.rsqrt(v + EPS)


def _gelu(x):
    c = math.sqrt(2.0 / math.pi)
    return 0.5 * x * (1.0 + jnp.tanh(c * (x + 0.044715 * (x * x * x))))


def _rb(x):
    return x.astype(BF16).astype(F32)


def _pack(x):
    return pltpu.bitcast(x.astype(BF16), U32)


def _unpack(x):
    return pltpu.bitcast(x, BF16)


def _dot(a, b):
    return jnp.dot(a, b, preferred_element_type=F32)


def _dot_nt(a, b):
    return lax.dot_general(a, b, (((1,), (1,)), ((), ())), preferred_element_type=F32)


def _kernel(x_hbm, wqkv_hbm, wo_hbm, win_hbm, wsp_hbm, bsp_hbm, wout_hbm, c_hbm, wmod_hbm,
            out_hbm,
            x_s, wqkv_s, wo_s, win_s, wsp_s, bsp_s, wout_s, c_s, wmod_s,
            mod_s, wqvt_s, k_s, qt_s, vt_s, ot_s, bad_s, s_s,
            x1_s, z1_s, z2_s, bcol_s, o_s,
            sem_in, sem_x, sem_out):
    def cp_in(src, dst, i):
        return pltpu.make_async_copy(src, dst, sem_in.at[i])

    cp_c = cp_in(c_hbm, c_s, 0)
    cp_wm1 = cp_in(wmod_hbm.at[:, 0:2 * D], wmod_s.at[:, 0:2 * D], 1)
    cp_wqkv = cp_in(wqkv_hbm, wqkv_s, 2)
    cp_wm2 = cp_in(wmod_hbm.at[:, 2 * D:6 * D], wmod_s.at[:, 2 * D:6 * D], 3)
    cp_wo = cp_in(wo_hbm, wo_s, 4)
    cp_win = cp_in(win_hbm, win_s, 5)
    cp_wsp = cp_in(wsp_hbm, wsp_s, 6)
    cp_bsp = cp_in(bsp_hbm, bsp_s, 7)
    cp_wout = cp_in(wout_hbm, wout_s, 8)

    def cp_x(r):
        return pltpu.make_async_copy(x_hbm.at[0, pl.ds(r * TP, TP), :],
                                     x_s.at[pl.ds(r * TP, TP), :], sem_x.at[r])

    cp_c.start()
    cp_wm1.start()
    cp_x(0).start()
    cp_wqkv.start()
    for r in range(1, S // TP):
        cp_x(r).start()

    cp_c.wait()
    cf = c_s[...].astype(F32)
    sc = jnp.broadcast_to((cf * jax.nn.sigmoid(cf)).astype(BF16), (16, D))
    cp_wm1.wait()
    mod_s[:, 0:2 * D] = _rb(_dot(sc, wmod_s[:, 0:2 * D]))[0:8]

    cp_wqkv.wait()
    wqvt_s[0:D // 2, :] = _pack(wqkv_s[:, 0:D].astype(F32).T)
    wqvt_s[D // 2:D, :] = _pack(wqkv_s[:, 2 * D:3 * D].astype(F32).T)
    q_scale = (DH ** -0.5) * math.log2(math.e)

    for r in range(S // TP):
        cp_x(r).wait()
    for cp in (cp_wm2, cp_wo, cp_win, cp_bsp, cp_wout, cp_wsp):
        cp.start()

    def proj(r, carry):
        r0 = pl.multiple_of(r * TP, TP)
        sa = mod_s[0:1, 0:D]
        ca1 = _rb(1.0 + mod_s[0:1, D:2 * D])
        h = (_ln(x_s[pl.ds(r0, TP), :].astype(F32)) * ca1 + sa).astype(BF16)
        k = _pack(_dot(h, wqkv_s[:, D:2 * D]))
        r2 = pl.multiple_of(r * (TP // 2), TP // 2)
        for b in range(D // 128):
            k_s[b, pl.ds(r2, TP // 2), :] = k[:, b * 128:(b + 1) * 128]
        qvt = _dot_nt(_unpack(wqvt_s[...]), h)
        qt_s[:, pl.ds(r0, TP)] = _pack(qvt[0:D] * q_scale)
        vt_s[:, pl.ds(r0, TP)] = _pack(qvt[D:2 * D])
        return carry

    lax.fori_loop(0, S // TP, proj, 0)

    def unit(u):
        h = u // NJ
        return dict(blk=h // 8,
                    shift=(128 - (h % 8) * DH) % 128,
                    r8=pl.multiple_of(h * 8, 8),
                    q0=pl.multiple_of((u % NJ) * TQ, TQ))

    def scores(d, qt, c, rev):
        ku = k_s[d["blk"], pl.ds(c * (CK // 2), CK // 2), :]
        if rev:
            ku = jnp.concatenate([ku[8 * g:8 * g + 8] for g in reversed(range(CK // 16))], axis=0)
        kk = _unpack(pltpu.roll(ku, d["shift"], 1))[:, 0:DH]
        return _dot(kk, qt)

    def pv(d, c, pb):
        return _dot(_unpack(vt_s[pl.ds(d["r8"], 8), pl.ds(c * CK, CK)]), pb)

    def attn_fast(i, carry):
        st = []
        for n in range(UN):
            d = unit(i * UN + n)
            d["qt"] = _unpack(qt_s[pl.ds(d["r8"], 8), pl.ds(d["q0"], TQ)])
            d["acc"] = jnp.zeros((DH, TQ), F32)
            d["l"] = jnp.zeros((8, TQ), F32)
            st.append(d)

        def finish(d, c, pb):
            d["acc"] = d["acc"] + pv(d, c, pb)
            if c == NC - 1:
                l = jnp.sum(d["l"], axis=0, keepdims=True)
                o = d["acc"] / l
                ok = jnp.logical_and(l >= L_LO, l <= L_HI)
                ok = jnp.logical_and(ok, jnp.abs(o) < jnp.inf)
                bad = jnp.where(ok, 0.0, 1.0)
                bad_s[...] = jnp.maximum(bad_s[...], bad)
                ot_s[pl.ds(d["r8"], 8), pl.ds(d["q0"], TQ)] = _pack(o)

        pend = []
        for d in st:
            for c in range(NC):
                p = jnp.exp2(scores(d, d["qt"], c, True))
                d["l"] = d["l"] + jnp.sum(p.reshape(CK // 8, 8, TQ), axis=0)
                p = jnp.concatenate([p[16 * g:16 * g + 16] for g in reversed(range(CK // 16))], axis=0)
                pend.append((d, c, p.astype(BF16)))
                if len(pend) > SKEW:
                    finish(*pend.pop(0))
        while pend:
            finish(*pend.pop(0))
        return carry

    bad_s[...] = jnp.zeros(bad_s.shape, F32)
    lax.fori_loop(0, H * NJ // UN, attn_fast, 0)

    def attn_exact(u, carry):
        d = unit(u)
        qt = _unpack(qt_s[pl.ds(d["r8"], 8), pl.ds(d["q0"], TQ)])

        def pass1(c, m):
            c0 = pl.multiple_of(c * CK, CK)
            ku = k_s[d["blk"], pl.ds(pl.multiple_of(c * (CK // 2), CK // 2), CK // 2), :]
            s = _dot(_unpack(pltpu.roll(ku, d["shift"], 1))[:, 0:DH], qt)
            s_s[pl.ds(c0, CK), :] = s
            return jnp.maximum(m, jnp.max(s, axis=0, keepdims=True))

        m = lax.fori_loop(0, NC, pass1, jnp.full((1, TQ), -jnp.inf, F32))

        def pass2(c, la):
            l, acc = la
            c0 = pl.multiple_of(c * CK, CK)
            p = jnp.exp2(s_s[pl.ds(c0, CK), :] - m)
            vt = _unpack(vt_s[pl.ds(d["r8"], 8), pl.ds(c0, CK)])
            return l + jnp.sum(p, axis=0, keepdims=True), acc + _dot(vt, p.astype(BF16))

        l, acc = lax.fori_loop(0, NC, pass2, (jnp.zeros((1, TQ), F32), jnp.zeros((DH, TQ), F32)))
        ot_s[pl.ds(d["r8"], 8), pl.ds(d["q0"], TQ)] = _pack(acc / l)
        return carry

    @pl.when(jnp.max(bad_s[...]) > 0.0)
    def _():
        lax.fori_loop(0, H * NJ, attn_exact, 0)

    cp_wm2.wait()
    mod_s[:, 2 * D:6 * D] = _rb(_dot(sc, wmod_s[:, 2 * D:6 * D]))[0:8]
    cp_bsp.wait()
    brow = bsp_s[...].reshape(1, S).astype(F32)
    for t in range(S // 128):
        bcol_s[t * 128:(t + 1) * 128, :] = jnp.broadcast_to(brow[:, t * 128:(t + 1) * 128], (128, 128)).T
    cp_wo.wait()
    cp_win.wait()

    def mix1(r, carry):
        r0 = pl.multiple_of(r * TM1, TM1)
        r2 = pl.multiple_of(r * (TM1 // 2), TM1 // 2)
        ga = mod_s[0:1, 2 * D:3 * D]
        sb = mod_s[0:1, 3 * D:4 * D]
        cb1 = _rb(1.0 + mod_s[0:1, 4 * D:5 * D])
        o = _unpack(ot_s[:, pl.ds(r0, TM1)]).astype(F32).T.astype(BF16)
        x1 = x_s[pl.ds(r0, TM1), :].astype(F32) + ga * _dot(o, wo_s[...])
        x1_s[pl.ds(r0, TM1), :] = x1
        h2 = (_ln(x1) * cb1 + sb).astype(BF16)
        z1_s[pl.ds(r0, TM1), :] = _gelu(_dot(h2, win_s[:, 0:FH]))
        z2_s[pl.ds(r2, TM1 // 2), :] = _pack(_ln(_gelu(_dot(h2, win_s[:, FH:2 * FH]))))
        return carry

    lax.fori_loop(0, S // TM1, mix1, 0)

    cp_wout.wait()
    cp_wsp.wait()

    def cp_out(t, slot):
        return pltpu.make_async_copy(o_s.at[slot], out_hbm.at[0, pl.ds(t * TM2, TM2), :], sem_out.at[slot])

    def mix2(t, carry):
        t0 = pl.multiple_of(t * TM2, TM2)
        slot = t % 2
        gb = mod_s[0:1, 5 * D:6 * D]
        g = _dot(wsp_s[pl.ds(t0, TM2), :], _unpack(z2_s[...]))
        b = bcol_s[pl.ds(t0, TM2), :]
        g = g + jnp.concatenate([b] * (FH // 128), axis=1)
        y = _dot((z1_s[pl.ds(t0, TM2), :] * g).astype(BF16), wout_s[...])
        res = (x1_s[pl.ds(t0, TM2), :] + gb * y).astype(BF16)

        @pl.when(t >= 2)
        def _():
            cp_out(t - 2, slot).wait()

        o_s[slot] = res
        cp_out(t, slot).start()
        return carry

    nt = S // TM2
    lax.fori_loop(0, nt, mix2, 0)
    cp_out(nt - 2, (nt - 2) % 2).wait()
    cp_out(nt - 1, (nt - 1) % 2).wait()


@jax.jit
def pallas_adaLN_cond__softmax_full_mha__mixer_gmlp__prompt_kernel(
    A_x: jax.Array,
    A_wqkv: jax.Array,
    A_wo: jax.Array,
    B_x: jax.Array,
    B_w_in: jax.Array,
    B_w_sp: jax.Array,
    B_b_sp: jax.Array,
    B_w_out: jax.Array,
    c: jax.Array,
    w_mod: jax.Array,
):
    del B_x
    hbm = pl.BlockSpec(memory_space=pl.ANY)
    scratch = [
        pltpu.VMEM((S, D), BF16),
        pltpu.VMEM((D, 3 * D), BF16),
        pltpu.VMEM((D, D), BF16),
        pltpu.VMEM((D, 2 * FH), BF16),
        pltpu.VMEM((S, S), BF16),
        pltpu.VMEM((S,), BF16),
        pltpu.VMEM((FH, D), BF16),
        pltpu.VMEM((1, D), BF16),
        pltpu.VMEM((D, 6 * D), BF16),
        pltpu.VMEM((8, 6 * D), F32),
        pltpu.VMEM((D, D), U32),
        pltpu.VMEM((D // 128, S // 2, 128), U32),
        pltpu.VMEM((D // 2, S), U32),
        pltpu.VMEM((D // 2, S), U32),
        pltpu.VMEM((D // 2, S), U32),
        pltpu.VMEM((DH, TQ), F32),
        pltpu.VMEM((S, TQ), F32),
        pltpu.VMEM((S, D), F32),
        pltpu.VMEM((S, FH), F32),
        pltpu.VMEM((S // 2, FH), U32),
        pltpu.VMEM((S, 128), F32),
        pltpu.VMEM((2, TM2, D), BF16),
        pltpu.SemaphoreType.DMA((9,)),
        pltpu.SemaphoreType.DMA((S // TP,)),
        pltpu.SemaphoreType.DMA((2,)),
    ]
    return pl.pallas_call(
        _kernel,
        out_shape=jax.ShapeDtypeStruct((1, S, D), BF16),
        in_specs=[hbm] * 9,
        out_specs=hbm,
        scratch_shapes=scratch,
        compiler_params=pltpu.CompilerParams(vmem_limit_bytes=100 * 1024 * 1024),
    )(A_x, A_wqkv, A_wo, B_w_in, B_w_sp, B_b_sp, B_w_out, c, w_mod)
```

```python
import math

import jax
import jax.numpy as jnp
from jax import lax
import jax.experimental.pallas as pl
import jax.experimental.pallas.tpu as pltpu

S = 2048
D = 512
H = 32
DH = 16
FH = 896
EPS = 1e-5

TQ = 512
NJ = S // TQ
CK = 128
NC = S // CK
HB = 2
POS = 7
DELTA = 2
LEAD = 0
RELD = 40
TP = 512
TM1 = 512
SM1 = 128
TM2 = 256
SM2 = 128

L_LO = 2.0 ** -60
L_HI = 2.0 ** 60

F32 = jnp.float32
BF16 = jnp.bfloat16
U32 = jnp.uint32


def _ln(x):
    m = jnp.mean(x, axis=-1, keepdims=True)
    xc = x - m
    v = jnp.mean(xc * xc, axis=-1, keepdims=True)
    return xc * lax.rsqrt(v + EPS)


def _gelu(x):
    c = math.sqrt(2.0 / math.pi)
    hx = 0.5 * x
    return hx + hx * jnp.tanh(x * (c + (c * 0.044715) * (x * x)))


def _rb(x):
    return x.astype(BF16).astype(F32)


def _pack(x):
    return pltpu.bitcast(x.astype(BF16), U32)


def _unpack(x):
    return pltpu.bitcast(x, BF16)


def _dot(a, b):
    return jnp.dot(a, b, preferred_element_type=F32)


def _dot_nt(a, b):
    return lax.dot_general(a, b, (((1,), (1,)), ((), ())), preferred_element_type=F32)


def _after(flag, x, dep):
    return jnp.where(flag, x, pltpu.bitcast(dep, U32))


def _bcast_k(ku, d):
    return _unpack(jnp.broadcast_to(ku[:, d:d + 1], (8, 128))).astype(F32)


def _kernel(x_hbm, wqkv_hbm, wo_hbm, win_hbm, wsp_hbm, bsp_hbm, wout_hbm, c_hbm, wmod_hbm,
            out_hbm,
            x_s, wqkv_s, wo_s, win_s, wsp_s, bsp_s, wout_s, c_s, wmod_s,
            mod_s, wqvt_s, h_s, k_s, kh_s, qt_s, vt_s, ot_s, kb0_s, kb1_s, qb0_s, qb1_s, bad_s, s_s,
            x1_s, z1_s, z2_s, bcol_s, o_s,
            sem_in, sem_x, sem_out):
    kbs = (kb0_s, kb1_s)
    qbs = (qb0_s, qb1_s)

    def cp_in(src, dst, i):
        return pltpu.make_async_copy(src, dst, sem_in.at[i])

    cp_c = cp_in(c_hbm, c_s.at[0], 0)
    cp_wm1 = cp_in(wmod_hbm.at[:, 0:2 * D], wmod_s.at[:, 0:2 * D], 1)
    cp_wk = cp_in(wqkv_hbm.at[:, D:2 * D], wqkv_s.at[:, D:2 * D], 2)
    cp_wm2 = cp_in(wmod_hbm.at[:, 2 * D:6 * D], wmod_s.at[:, 2 * D:6 * D], 3)
    cp_wo = cp_in(wo_hbm, wo_s, 4)
    cp_win = cp_in(win_hbm, win_s, 5)
    cp_wsp = cp_in(wsp_hbm, wsp_s, 6)
    cp_bsp = cp_in(bsp_hbm, bsp_s.at[0:S], 7)
    cp_wout = cp_in(wout_hbm, wout_s, 8)
    cp_wq = cp_in(wqkv_hbm.at[:, 0:D], wqkv_s.at[:, 0:D], 9)
    cp_wv = cp_in(wqkv_hbm.at[:, 2 * D:3 * D], wqkv_s.at[:, 2 * D:3 * D], 10)

    def cp_x(r):
        return pltpu.make_async_copy(x_hbm.at[0, pl.ds(r * TP, TP), :],
                                     x_s.at[pl.ds(r * TP, TP), :], sem_x.at[r])

    cp_c.start()
    cp_wm1.start()
    cp_x(0).start()
    cp_wk.start()

    cp_c.wait()
    cf = c_s[0].astype(F32)
    sc = jnp.broadcast_to((cf * jax.nn.sigmoid(cf)).astype(BF16), (16, D))
    cp_x(0).wait()
    cp_x(1).start()
    cp_wq.start()
    cp_wv.start()
    n0 = _ln(x_s[0:TP, :].astype(F32))
    cp_wm1.wait()
    mod1 = _rb(_dot(sc, wmod_s[:, 0:2 * D]))[0:1]
    sa = mod1[:, 0:D]
    ca1 = _rb(1.0 + mod1[:, D:2 * D])

    q_scale = (DH ** -0.5) * math.log2(math.e)

    def make_h(r, n):
        h = (n * ca1 + sa).astype(BF16)
        h_s[r * (TP // 2):(r + 1) * (TP // 2), :] = pltpu.bitcast(h, U32)
        return h

    def ln_x(r):
        return _ln(x_s[r * TP:(r + 1) * TP, :].astype(F32))

    def proj_k(r, h):
        k_s[r * (TP // 2):(r + 1) * (TP // 2), :] = _pack(_dot(h, wqkv_s[:, D:2 * D]))

    h0 = make_h(0, n0)
    cp_wk.wait()
    cp_x(2).start()
    cp_x(3).start()
    cp_x(1).wait()
    proj_k(0, h0)
    h1 = make_h(1, ln_x(1))
    cp_x(2).wait()
    cp_wq.wait()
    cp_wv.wait()
    cp_x(3).wait()
    for cp in (cp_wm2, cp_bsp, cp_wo, cp_win, cp_wout, cp_wsp):
        cp.start()
    proj_k(1, h1)
    h2 = make_h(2, ln_x(2))
    proj_k(2, h2)
    h3 = make_h(3, ln_x(3))
    proj_k(3, h3)
    wqvt_s[0:D // 2, :] = _pack(wqkv_s[:, 0:D].astype(F32).T)
    wqvt_s[D // 2:D, :] = _pack(wqkv_s[:, 2 * D:3 * D].astype(F32).T)

    def proj_qv(r, carry):
        rows = pl.ds(pl.multiple_of(r * (TP // 2), TP // 2), TP // 2)
        cols = pl.ds(pl.multiple_of(r * TP, TP), TP)
        qvt = _dot_nt(_unpack(wqvt_s[...]), _unpack(h_s[rows, :]))
        q = (qvt[0:D] * q_scale).astype(BF16)
        qt_s[:, cols] = pltpu.bitcast(q, U32)
        vt_s[:, cols] = _pack(qvt[D:2 * D])
        q0 = q[0:DH].astype(F32)
        for d in range(DH):
            qb0_s[d * 8:(d + 1) * 8, cols] = jnp.broadcast_to(q0[d:d + 1], (8, TP))
        k = k_s[rows, :]
        for b in range(D // 128):
            kblk = k[:, b * 128:(b + 1) * 128]
            for j in range(8):
                kh_s[b * 8 + j, rows, :] = kblk if j == 0 else pltpu.roll(kblk, 128 - j * DH, 1)
        for t in range(TP // CK):
            ku = k[t * 64 + POS * 8:t * 64 + POS * 8 + 8, 0:128]
            trow = pl.ds(pl.multiple_of(r * (16 * TP // CK) + 16 * t, 16), 16)
            for d in range(DH):
                kb0_s[trow, d * 128:(d + 1) * 128] = _bcast_k(ku, d)
        return carry

    lax.fori_loop(0, S // TP, proj_qv, 0)

    cp_wm2.wait()
    cp_bsp.wait()
    mod_s[...] = _rb(_dot(sc, wmod_s[:, 2 * D:6 * D]))[0:8]
    brow = bsp_s[0:S].reshape(1, S).astype(F32)
    for t in range(S // 128):
        bcol_s[t * 128:(t + 1) * 128, :] = jnp.broadcast_to(brow[:, t * 128:(t + 1) * 128], (128, 128)).T
    bad_s[...] = jnp.zeros(bad_s.shape, F32)

    def attn_fast(i, carry):
        zsrc = qt_s[0:8, 0:128]
        yes = [(zsrc & (1 << b)) <= (1 << b) for b in range(4)]
        st = []
        for un in range(HB * NJ):
            h = i * HB + un // NJ
            r8 = pl.multiple_of(h * 8, 8)
            q0 = (un % NJ) * TQ
            st.append(dict(h=h, r8=r8, q0=q0, kb=kbs[(un // NJ) % 2], qb=qbs[(un // NJ) % 2],
                           qt=_unpack(qt_s[pl.ds(r8, 8), q0:q0 + TQ]),
                           acc=jnp.zeros((DH, TQ), F32), l=jnp.zeros((8, TQ), F32),
                           grp={}, pc={}))

        def piece(d, t, half, jj):
            r0 = t * 16 + half * 8
            c0 = d["q0"] + jj * 128
            a = [None, None]
            for dd in range(DH):
                m = d["kb"][r0:r0 + 8, dd * 128:(dd + 1) * 128] * d["qb"][dd * 8:(dd + 1) * 8, c0:c0 + 128]
                a[dd % 2] = m if a[dd % 2] is None else a[dd % 2] + m
            s = a[0] + a[1]
            d["pc"][(t, half, jj)] = jnp.exp2(s)
            return s

        def pv(d, t):
            top = jnp.concatenate([d["pc"][(t, 0, jj)] for jj in range(TQ // 128)], axis=1)
            bot = jnp.concatenate([d["pc"][(t, 1, jj)] for jj in range(TQ // 128)], axis=1)
            d["l"] = d["l"] + (top + bot)
            d["grp"][(t, POS)] = jnp.concatenate([top, bot], axis=0)
            p = jnp.concatenate([d["grp"][(t, r)] for r in range(8)], axis=0)
            vt = _unpack(vt_s[pl.ds(d["r8"], 8), t * CK:(t + 1) * CK])
            d["acc"] = d["acc"] + _dot(vt, p.astype(BF16))
            if t == NC - 1:
                l = jnp.sum(d["l"], axis=0, keepdims=True)
                o = d["acc"] / l
                ok = jnp.logical_and(l >= L_LO, l <= L_HI)
                ok = jnp.logical_and(ok, jnp.abs(o) < jnp.inf)
                bad_s[...] = jnp.maximum(bad_s[...], jnp.where(ok, 0.0, 1.0))
                ot_s[pl.ds(d["r8"], 8), d["q0"]:d["q0"] + TQ] = _pack(o)

        stream, tile_end, tiles = [], [], []
        for d in st:
            for t in range(NC):
                stream += [(d, t, r) for r in reversed(range(8)) if r != POS]
                tile_end.append(len(stream))
                tiles.append((d, t))
        pv_at, pv_pos = {}, []
        for ti in range(len(tiles)):
            pos = min(tile_end[ti + 1] + DELTA, len(stream)) if ti + 1 < len(tiles) else len(stream)
            pv_pos.append(pos)
            pv_at.setdefault(pos, []).append(ti)
        ties = {}
        prev_end = -1
        for ti in range(len(tiles)):
            end = max((pv_pos[ti - 1] if ti > 0 else 8) - LEAD, prev_end + 1)
            span = end - prev_end
            for n in range(8):
                pos = prev_end + 1 + (n * span) // 8 if span < 8 else end - 7 + n
                ties.setdefault(min(pos, len(stream) - 1), []).append(("pc", ti, n % 2, n // 2))
            prev_end = end
        per_head = 7 * NC * NJ
        lo_g, span_g = RELD + 2, per_head - RELD - 18
        for hh in range(HB):
            for n in range(NC * DH):
                ties.setdefault(hh * per_head + lo_g + (n * span_g) // (NC * DH), []).append(
                    ("kb", hh, n % NC, n // NC))
            for n in range(64):
                ties.setdefault(hh * per_head + lo_g + 1 + (n * span_g) // 64, []).append(
                    ("qb", hh, n // 4, n % 4))
        cuts = set(pv_at) | {0, len(stream)}
        cuts |= {a for a in range(1, len(stream)) if stream[a][0] is not stream[a - 1][0]}
        cuts = sorted(cuts)

        hist = {}
        for lo, hi in zip(cuts[:-1], cuts[1:]):
            d = stream[lo][0]
            parts = []
            for n in range(lo, hi):
                _, t, r = stream[n]
                kv = kh_s[d["h"], pl.ds(t * 64 + r * 8, 8), :]
                for tn, tie in enumerate(ties.get(n, [])):
                    if tie[0] == "pc":
                        val = piece(*tiles[tie[1]], tie[2], tie[3])
                    else:
                        hn = jnp.minimum(i * HB + tie[1] + 1, H - 1)
                        if tie[0] == "kb":
                            _, hh, tt, dd = tie
                            src = _after(yes[0], kh_s[hn, pl.ds(tt * 64 + POS * 8, 8), :], hist[n - RELD])
                            val = _bcast_k(src, dd)
                            kbs[(hh + 1) % 2][16 * tt:16 * tt + 16, dd * 128:(dd + 1) * 128] = val
                            val = val[8:16]
                        else:
                            _, hh, col, dq = tie
                            src = qt_s[pl.ds(pl.multiple_of(hn * 8, 8), 8), col * 128:(col + 1) * 128]
                            qf = _unpack(_after(yes[0], src, hist[n - RELD])).astype(F32)
                            for dd in range(dq * 4, dq * 4 + 4):
                                val = jnp.broadcast_to(qf[dd:dd + 1, :], (8, 128))
                                qbs[(hh + 1) % 2][dd * 8:(dd + 1) * 8, col * 128:(col + 1) * 128] = val
                    kv = _after(yes[tn], kv, val)
                parts.append(kv)
            kk = _unpack(jnp.concatenate(parts, axis=0))[:, 0:DH]
            p = jnp.exp2(_dot(kk, d["qt"]))
            d["l"] = d["l"] + jnp.sum(p.reshape(2 * (hi - lo), 8, TQ), axis=0)
            for n in range(lo, hi):
                _, t, r = stream[n]
                d["grp"][(t, r)] = p[16 * (n - lo):16 * (n - lo) + 16]
                hist[n] = p[16 * (n - lo):16 * (n - lo) + 8, 0:128]
            for ti in pv_at.get(hi, []):
                pv(*tiles[ti])
        return carry

    lax.fori_loop(0, H // HB, attn_fast, 0)

    def attn_exact(u, carry):
        h = u // NJ
        r8 = pl.multiple_of(h * 8, 8)
        q0 = pl.multiple_of((u % NJ) * TQ, TQ)
        qt = _unpack(qt_s[pl.ds(r8, 8), pl.ds(q0, TQ)])

        def pass1(c, m):
            ku = kh_s[h, pl.ds(pl.multiple_of(c * (CK // 2), CK // 2), CK // 2), :]
            s = _dot(_unpack(ku)[:, 0:DH], qt)
            s_s[pl.ds(pl.multiple_of(c * CK, CK), CK), :] = s
            return jnp.maximum(m, jnp.max(s, axis=0, keepdims=True))

        m = lax.fori_loop(0, NC, pass1, jnp.full((1, TQ), -jnp.inf, F32))

        def pass2(c, la):
            l, acc = la
            c0 = pl.multiple_of(c * CK, CK)
            p = jnp.exp2(s_s[pl.ds(c0, CK), :] - m)
            vt = _unpack(vt_s[pl.ds(r8, 8), pl.ds(c0, CK)])
            return l + jnp.sum(p, axis=0, keepdims=True), acc + _dot(vt, p.astype(BF16))

        l, acc = lax.fori_loop(0, NC, pass2, (jnp.zeros((1, TQ), F32), jnp.zeros((DH, TQ), F32)))
        ot_s[pl.ds(r8, 8), pl.ds(q0, TQ)] = _pack(acc / l)
        return carry

    @pl.when(jnp.max(bad_s[...]) > 0.0)
    def _():
        lax.fori_loop(0, H * NJ, attn_exact, 0)

    cp_wo.wait()
    cp_win.wait()

    def mix1(r, carry):
        ga = mod_s[0:1, 0:D]
        sb = mod_s[0:1, D:2 * D]
        cb1 = _rb(1.0 + mod_s[0:1, 2 * D:3 * D])

        def stage_a(n):
            r0 = pl.multiple_of(r * TM1 + n * SM1, SM1)
            o = _unpack(ot_s[:, pl.ds(r0, SM1)]).astype(F32).T.astype(BF16)
            x1 = x_s[pl.ds(r0, SM1), :].astype(F32) + ga * _dot(o, wo_s[...])
            x1_s[pl.ds(r0, SM1), :] = x1
            return (_ln(x1) * cb1 + sb).astype(BF16)

        def stage_b(n, h2):
            r0 = pl.multiple_of(r * TM1 + n * SM1, SM1)
            r2 = pl.multiple_of(r * (TM1 // 2) + n * (SM1 // 2), SM1 // 2)
            z2_s[pl.ds(r2, SM1 // 2), :] = _pack(_ln(_gelu(_dot(h2, win_s[:, FH:2 * FH]))))
            z1_s[pl.ds(r0, SM1), :] = _gelu(_dot(h2, win_s[:, 0:FH]))

        ns = TM1 // SM1
        h2 = [stage_a(0), stage_a(1)]
        for n in range(ns):
            if n + 2 < ns:
                h2.append(stage_a(n + 2))
            stage_b(n, h2[n])
        return carry

    lax.fori_loop(0, S // TM1, mix1, 0)

    cp_wout.wait()
    cp_wsp.wait()

    def cp_out(t, slot):
        return pltpu.make_async_copy(o_s.at[slot], out_hbm.at[0, pl.ds(t * TM2, TM2), :], sem_out.at[slot])

    def mix2(t, carry):
        slot = t % 2
        gb = mod_s[0:1, 3 * D:4 * D]

        @pl.when(t >= 2)
        def _():
            cp_out(t - 2, slot).wait()

        def gate(n):
            t0 = pl.multiple_of(t * TM2 + n * SM2, SM2)
            g = _dot(wsp_s[pl.ds(t0, SM2), :], _unpack(z2_s[...]))
            b = bcol_s[pl.ds(t0, SM2), :]
            g = g + jnp.concatenate([b] * (FH // 128), axis=1)
            return (z1_s[pl.ds(t0, SM2), :] * g).astype(BF16)

        def proj_out(n, u):
            t0 = pl.multiple_of(t * TM2 + n * SM2, SM2)
            res = x1_s[pl.ds(t0, SM2), :] + gb * _dot(u, wout_s[...])
            o_s[slot, n * SM2:(n + 1) * SM2, :] = res.astype(BF16)

        ns = TM2 // SM2
        u = [gate(n) for n in range(ns)]
        for n in range(ns):
            proj_out(n, u[n])
        cp_out(t, slot).start()
        return carry

    nt = S // TM2
    lax.fori_loop(0, nt, mix2, 0)
    cp_out(nt - 2, (nt - 2) % 2).wait()
    cp_out(nt - 1, (nt - 1) % 2).wait()


@jax.jit
def pallas_adaLN_cond__softmax_full_mha__mixer_gmlp__prompt_kernel(
    A_x: jax.Array,
    A_wqkv: jax.Array,
    A_wo: jax.Array,
    B_x: jax.Array,
    B_w_in: jax.Array,
    B_w_sp: jax.Array,
    B_b_sp: jax.Array,
    B_w_out: jax.Array,
    c: jax.Array,
    w_mod: jax.Array,
):
    del B_x
    hbm = pl.BlockSpec(memory_space=pl.ANY)
    scratch = [
        pltpu.VMEM((S, D), BF16),
        pltpu.VMEM((D, 3 * D), BF16),
        pltpu.VMEM((D, D), BF16),
        pltpu.VMEM((D, 2 * FH), BF16),
        pltpu.VMEM((S, S), BF16),
        pltpu.VMEM((4 * S,), BF16),
        pltpu.VMEM((FH, D), BF16),
        pltpu.VMEM((8, 1, D), BF16),
        pltpu.VMEM((D, 6 * D), BF16),
        pltpu.VMEM((8, 4 * D), F32),
        pltpu.VMEM((D, D), U32),
        pltpu.VMEM((S // 2, D), U32),
        pltpu.VMEM((S // 2, D), U32),
        pltpu.VMEM((H, S // 2, 128), U32),
        pltpu.VMEM((D // 2, S), U32),
        pltpu.VMEM((D // 2, S), U32),
        pltpu.VMEM((D // 2, S), U32),
        pltpu.VMEM((NC * 16, DH * 128), F32),
        pltpu.VMEM((NC * 16, DH * 128), F32),
        pltpu.VMEM((DH * 8, S), F32),
        pltpu.VMEM((DH * 8, S), F32),
        pltpu.VMEM((DH, TQ), F32),
        pltpu.VMEM((S, TQ), F32),
        pltpu.VMEM((S, D), F32),
        pltpu.VMEM((S, FH), F32),
        pltpu.VMEM((S // 2, FH), U32),
        pltpu.VMEM((S, 128), F32),
        pltpu.VMEM((2, TM2, D), BF16),
        pltpu.SemaphoreType.DMA((11,)),
        pltpu.SemaphoreType.DMA((S // TP,)),
        pltpu.SemaphoreType.DMA((2,)),
    ]
    return pl.pallas_call(
        _kernel,
        out_shape=jax.ShapeDtypeStruct((1, S, D), BF16),
        in_specs=[hbm] * 9,
        out_specs=hbm,
        scratch_shapes=scratch,
        compiler_params=pltpu.CompilerParams(vmem_limit_bytes=110 * 1024 * 1024),
    )(A_x, A_wqkv, A_wo, B_w_in, B_w_sp, B_b_sp, B_w_out, c, w_mod)
```

```python
import math

import jax
import jax.numpy as jnp
from jax import lax
import jax.experimental.pallas as pl
import jax.experimental.pallas.tpu as pltpu

S = 2048
D = 512
H = 32
DH = 16
FH = 896
EPS = 1e-5

TQ = 512
NJ = S // TQ
CK = 128
NC = S // CK
HB = 2
POS = 0
DELTA = 2
LEAD = 5
CW = 8
RELD = 40
SP = 256
PACE_LO = 0.25
PACE_HI = 0.98
TP = 512
TM1 = 512
SM1 = 128
TM2 = 256
SM2 = 128

L_LO = 2.0 ** -60
L_HI = 2.0 ** 60
V_HI = 2.0 ** 60

F32 = jnp.float32
BF16 = jnp.bfloat16
U32 = jnp.uint32


def _ln(x):
    m = jnp.mean(x, axis=-1, keepdims=True)
    xc = x - m
    v = jnp.mean(xc * xc, axis=-1, keepdims=True)
    return xc * lax.rsqrt(v + EPS)


def _gelu(x):
    c = math.sqrt(2.0 / math.pi)
    hx = 0.5 * x
    return hx + hx * jnp.tanh(x * (c + (c * 0.044715) * (x * x)))


def _rb(x):
    return x.astype(BF16).astype(F32)


def _pack(x):
    return pltpu.bitcast(x.astype(BF16), U32)


def _unpack(x):
    return pltpu.bitcast(x, BF16)


def _dot(a, b):
    return jnp.dot(a, b, preferred_element_type=F32)


def _dot_nt(a, b):
    return lax.dot_general(a, b, (((1,), (1,)), ((), ())), preferred_element_type=F32)


def _after(flag, x, dep):
    return jnp.where(flag, x, pltpu.bitcast(dep, U32))


def _paced_dot(flag, lhs, w, deps, lo, hi):
    ng, nn = lhs.shape[0] // 8, w.shape[1] // 128
    at = {}
    for n, row in enumerate(deps):
        idx = int((lo + (hi - lo) * n / max(len(deps) - 1, 1)) * ng * nn)
        at.setdefault(min(idx, ng * nn - 1), []).append(row)
    outs = []
    for j in range(nn):
        col0 = []
        for g in range(ng):
            v = lhs[8 * g:8 * g + 8, 0:128]
            rows = at.get(j * ng + g, [])
            if rows:
                fold = None
                for row in rows:
                    for k in range(row.shape[1] // 128):
                        part = row[:, 128 * k:128 * k + 128]
                        fold = part if fold is None else fold | part
                v = jnp.where(flag, v, fold)
            col0.append(v)
        lj = jnp.concatenate([jnp.concatenate(col0, axis=0), lhs[:, 128:]], axis=1)
        outs.append(_dot(_unpack(lj), w[:, 128 * j:128 * j + 128]))
    return jnp.concatenate(outs, axis=1)


def _row_blocks(x):
    return [x[8 * n:8 * n + 8] for n in range(x.shape[0] // 8)]


def _bcast_k(ku, d):
    return _unpack(jnp.broadcast_to(ku[:, d:d + 1], (8, 128))).astype(F32)


def _kernel(x_hbm, wqkv_hbm, wo_hbm, win_hbm, wsp_hbm, bsp_hbm, wout_hbm, c_hbm, wmod_hbm,
            out_hbm,
            x_s, wqkv_s, wo_s, win_s, wsp_s, bsp_s, wout_s, c_s, wmod_s,
            mod_s, sc_s, brow_s, wqvt_s, h_s, k_s, kh_s, qt_s, vt_s, ot_s, kb0_s, kb1_s, qb0_s, qb1_s, chk_s, carp_s, cara_s, s_s,
            x1_s, z1_s, z2_s, bcol_s, o_s,
            sem_in, sem_x, sem_m, sem_out):
    kbs = (kb0_s, kb1_s)
    qbs = (qb0_s, qb1_s)

    def cp_in(src, dst, i):
        return pltpu.make_async_copy(src, dst, sem_in.at[i])

    cp_c = cp_in(c_hbm, c_s.at[0], 0)
    cp_wm1 = cp_in(wmod_hbm.at[:, 0:2 * D], wmod_s.at[:, 0:2 * D], 1)
    cp_wk = cp_in(wqkv_hbm.at[:, D:2 * D], wqkv_s.at[:, D:2 * D], 2)
    cp_wo = cp_in(wo_hbm, wo_s, 4)
    cp_win = cp_in(win_hbm, win_s, 5)
    cp_wsp = cp_in(wsp_hbm, wsp_s, 6)
    cp_bsp = cp_in(bsp_hbm, bsp_s.at[0:S], 7)
    cp_wout = cp_in(wout_hbm, wout_s, 8)
    cp_wq = cp_in(wqkv_hbm.at[:, 0:D], wqkv_s.at[:, 0:D], 9)
    cp_wv = cp_in(wqkv_hbm.at[:, 2 * D:3 * D], wqkv_s.at[:, 2 * D:3 * D], 10)

    xb = (0, 1, 2, 4, 8)

    def cp_x(r):
        rows = pl.ds(xb[r] * SP, (xb[r + 1] - xb[r]) * SP)
        return pltpu.make_async_copy(x_hbm.at[0, rows, :], x_s.at[rows, :], sem_x.at[r])

    def cp_wm2(r):
        cols = pl.ds(pl.multiple_of((2 + r) * D, D), D)
        return pltpu.make_async_copy(wmod_hbm.at[:, cols], wmod_s.at[:, cols], sem_m.at[r])

    cp_c.start()
    cp_wm1.start()
    cp_x(0).start()

    cp_c.wait()
    cp_wk.start()
    cp_x(1).start()
    cf = c_s[0].astype(F32)
    sc = jnp.broadcast_to((cf * jax.nn.sigmoid(cf)).astype(BF16), (16, D))
    sc_s[...] = pltpu.bitcast(sc, U32)
    cp_x(0).wait()
    n0 = _ln(x_s[0:SP, :].astype(F32))
    cp_wm1.wait()
    cp_x(2).start()
    mod1 = _rb(_dot(sc, wmod_s[:, 0:2 * D]))[0:1]
    sa = mod1[:, 0:D]
    ca1 = _rb(1.0 + mod1[:, D:2 * D])

    q_scale = (DH ** -0.5) * math.log2(math.e)
    zsrc0 = pltpu.bitcast(sc, U32)[:, 0:128]
    yes0 = (zsrc0 & 1) <= 1

    def make_h(j, n=None):
        if n is None:
            n = _ln(x_s[j * SP:(j + 1) * SP, :].astype(F32))
        hu = _pack(n * ca1 + sa)
        h_s[j * (SP // 2):(j + 1) * (SP // 2), :] = hu
        return hu

    def proj_k(j, hu, dep=None):
        k = _paced_dot(yes0, hu, wqkv_s[:, D:2 * D], _row_blocks(dep), PACE_LO, PACE_HI)
        k_s[j * (SP // 2):(j + 1) * (SP // 2), :] = _pack(k)

    hs = {0: make_h(0, n0)}
    cp_wk.wait()
    cp_x(1).wait()
    cp_x(3).start()
    hs[1] = make_h(1)
    proj_k(0, hs[0], hs[1])
    cp_x(2).wait()
    cp_wq.start()
    cp_wv.start()
    hs[2] = make_h(2)
    proj_k(1, hs[1], hs[2])
    hs[3] = make_h(3)
    proj_k(2, hs[2], hs[3])
    cp_x(3).wait()
    for r in range(4):
        cp_wm2(r).start()
    cp_bsp.start()
    hs[4] = make_h(4)
    proj_k(3, hs[3], hs[4])
    hs[5] = make_h(5)
    proj_k(4, hs[4], hs[5])
    hs[6] = make_h(6)
    proj_k(5, hs[5], hs[6])
    cp_wq.wait()
    cp_wv.wait()
    for cp in (cp_wo, cp_win, cp_wout, cp_wsp):
        cp.start()
    hs[7] = make_h(7)
    wqt = _pack(wqkv_s[:, 0:D].astype(F32).T)
    wqvt_s[0:D // 2, :] = wqt
    proj_k(6, hs[6], jnp.concatenate([hs[7], wqt], axis=0))
    wvt = _pack(wqkv_s[:, 2 * D:3 * D].astype(F32).T)
    wqvt_s[D // 2:D, :] = wvt
    proj_k(7, hs[7], wvt)
    chk_s[0:16, :] = jnp.ones((16, TQ), F32)
    chk_s[16:24, :] = jnp.zeros((8, TQ), F32)
    carp_s[...] = jnp.zeros(carp_s.shape, F32)
    cara_s[...] = jnp.zeros(cara_s.shape, F32)
    kb1_s[2 * NC - 2:2 * NC] = jnp.zeros((2, DH * 8, 128), F32)
    qb1_s[:, S - TQ:S] = jnp.zeros((DH * 8, TQ), F32)
    cp_bsp.wait()
    brow_s[...] = jnp.broadcast_to(bsp_s[0:S].reshape(1, S).astype(F32), (8, S))

    def proj_qv(r, carry):
        rows = pl.ds(pl.multiple_of(r * (TP // 2), TP // 2), TP // 2)
        cols = pl.ds(pl.multiple_of(r * TP, TP), TP)
        cp_wm2(r).wait()
        qvt = _dot_nt(_unpack(wqvt_s[...]), _unpack(h_s[rows, :]))
        q = (qvt[0:D] * q_scale).astype(BF16)
        qt_s[:, cols] = pltpu.bitcast(q, U32)
        vt_s[:, cols] = _pack(qvt[D:2 * D])
        vmax = jnp.max(jnp.abs(qvt[D:2 * D]).reshape(D // 8, 8, TP), axis=0)
        chk_s[16:24, :] = jnp.maximum(chk_s[16:24, :], vmax)
        q0 = q[0:DH].astype(F32)
        for d in range(DH):
            qb0_s[d * 8:(d + 1) * 8, cols] = jnp.broadcast_to(q0[d:d + 1], (8, TP))
        k = k_s[rows, :]
        for b in range(D // 128):
            kblk = k[:, b * 128:(b + 1) * 128]
            for j in range(8):
                kh_s[b * 8 + j, rows, :] = kblk if j == 0 else pltpu.roll(kblk, 128 - j * DH, 1)
        for t in range(TP // CK):
            ku = k[t * 64 + POS * 8:t * 64 + POS * 8 + 8, 0:128]
            tg = r * (2 * TP // CK) + 2 * t
            for d in range(DH):
                val = _bcast_k(ku, d)
                kb0_s[tg, d * 8:(d + 1) * 8, :] = val[0:8]
                kb0_s[tg + 1, d * 8:(d + 1) * 8, :] = val[8:16]
        mcols = pl.ds(pl.multiple_of((2 + r) * D, D), D)
        mod_s[:, pl.ds(pl.multiple_of(r * D, D), D)] = _rb(_dot(_unpack(sc_s[...]), wmod_s[:, mcols]))[0:8]
        brow = brow_s[0:1, cols]
        for t in range(TP // 128):
            trow = pl.ds(pl.multiple_of(r * TP + t * 128, 128), 128)
            bcol_s[trow, :] = jnp.broadcast_to(brow[:, t * 128:(t + 1) * 128], (128, 128)).T
        return carry

    lax.fori_loop(0, S // TP, proj_qv, 0)

    nt_body = HB * NJ * NC

    def vpu_scores(d, t, half, jj):
        c0 = d["q0"] + jj * 128
        m = d["kb"][2 * t + half] * d["qb"][:, c0:c0 + 128]
        return jnp.sum(jnp.sum(m.reshape(DH // 2, 2, 8, 128), axis=0), axis=0)

    def vpu_group(d, t):
        top = jnp.concatenate([d["pc"][(t, 0, jj)] for jj in range(TQ // 128)], axis=1)
        bot = jnp.concatenate([d["pc"][(t, 1, jj)] for jj in range(TQ // 128)], axis=1)
        d["l"] = d["l"] + (top + bot)
        d["grp"][(t, POS)] = jnp.concatenate([top, bot], axis=0)

    def pv_dot(d, t, vt):
        p = jnp.concatenate([d["grp"][(t, r)] for r in range(8)], axis=0)
        d["acc"] = d["acc"] + _dot(_unpack(vt), p.astype(BF16))

    def finish(d):
        l = jnp.sum(d["l"], axis=0, keepdims=True)
        chk_s[0:1, :] = jnp.minimum(chk_s[0:1, :], l)
        chk_s[8:9, :] = jnp.maximum(chk_s[8:9, :], l)
        ot_s[pl.ds(d["o8"], 8), d["q0"]:d["q0"] + TQ] = _pack(d["acc"] * (1.0 / l))

    def carried_unit(h_prev, o8):
        d = dict(r8=pl.multiple_of(h_prev * 8, 8), o8=o8, q0=(NJ - 1) * TQ,
                 kb=kbs[(HB - 1) % 2], qb=qbs[(HB - 1) % 2],
                 acc=cara_s[0:DH, :], l=cara_s[DH:DH + 8, :], grp={}, pc={})
        for r in range(8):
            d["grp"][(NC - 2, r)] = carp_s[16 * r:16 * r + 16, :]
            if r != POS:
                d["grp"][(NC - 1, r)] = carp_s[CK + 16 * r:CK + 16 * r + 16, :]
        return d

    def attn_fast(i, carry):
        zsrc = qt_s[0:8, 0:128]
        yes = [(zsrc & (1 << b)) <= (1 << b) for b in range(4)]
        st = []
        for un in range(HB * NJ):
            h = i * HB + un // NJ
            r8 = pl.multiple_of(h * 8, 8)
            q0 = (un % NJ) * TQ
            st.append(dict(h=h, r8=r8, o8=r8, q0=q0, kb=kbs[(un // NJ) % 2], qb=qbs[(un // NJ) % 2],
                           qt=_unpack(qt_s[pl.ds(r8, 8), q0:q0 + TQ]),
                           acc=jnp.zeros((DH, TQ), F32), l=jnp.zeros((8, TQ), F32),
                           grp={}, pc={}))
        hp = jnp.maximum(i * HB - 1, 0)
        dc = carried_unit(hp, pl.multiple_of(jnp.where(i == 0, H * 8, hp * 8), 8))

        stream, tile_end = [], []
        tiles = {-2: (dc, NC - 2), -1: (dc, NC - 1)}
        for un, d in enumerate(st):
            for t in range(NC):
                stream += [(d, t, r) for r in reversed(range(8)) if r != POS]
                tile_end.append(len(stream))
                tiles[un * NC + t] = (d, t)
        pv_at = {(tile_end[ti + 1] if ti + 1 >= 0 else 0) + DELTA: ti for ti in range(-2, nt_body - 2)}
        slots, slot_of_pv = [], {}
        for n in range(len(stream)):
            if n in pv_at:
                slot_of_pv[pv_at[n]] = len(slots)
                slots.append(("v", pv_at[n]))
            slots.append(("k", n))
        ties = {}
        prev_end = -1
        for ti in range(-1, nt_body - 1):
            end = CW if ti == -1 else slot_of_pv[ti] - LEAD if ti in slot_of_pv else len(slots) - 1
            span = end - prev_end
            for n in range(8):
                pos = prev_end + 1 + (n * span) // 8 if span < 8 else end - ((7 - n) * span) // 8
                ties.setdefault(slots[pos], []).append(("pc", ti, n % 2, n // 2))
            prev_end = end
        per_head = len(stream) // HB
        lo_g, span_g = RELD + 2, per_head - RELD - 18
        kgroups = [(t, b) for b in range(0, DH, 2) for t in range(NC)]
        qgroups = [(col, b) for col in range(S // 128) for b in range(0, DH, 4)]
        for hh in range(HB):
            for n, g in enumerate(kgroups):
                ties.setdefault(("k", hh * per_head + lo_g + (n * span_g) // len(kgroups)), []).append(
                    ("kb", hh) + g)
            for n, g in enumerate(qgroups):
                ties.setdefault(("k", hh * per_head + lo_g + 1 + (n * span_g) // len(qgroups)), []).append(
                    ("qb", hh) + g)
        cuts = set(pv_at) | {0, len(stream)}
        cuts |= {a for a in range(1, len(stream)) if stream[a][0] is not stream[a - 1][0]}
        cuts = sorted(cuts)
        hist = {}

        def side_work(tie, n):
            if tie[0] == "pc":
                _, ti, half, jj = tie
                d, t = tiles[ti]
                s = vpu_scores(d, t, half, jj)
                d["pc"][(t, half, jj)] = jnp.exp2(s)
                return s
            hn = jnp.minimum(i * HB + tie[1] + 1, H - 1)
            if tie[0] == "kb":
                _, hh, tt, b = tie
                src = _after(yes[0], kh_s[hn, pl.ds(tt * 64 + POS * 8, 8), :], hist[n - RELD])
                for dd in range(b, b + 2):
                    val = _bcast_k(src, dd)
                    kbs[(hh + 1) % 2][2 * tt, dd * 8:(dd + 1) * 8, :] = val[0:8]
                    val = val[8:16]
                    kbs[(hh + 1) % 2][2 * tt + 1, dd * 8:(dd + 1) * 8, :] = val
                return val
            _, hh, col, b = tie
            src = qt_s[pl.ds(pl.multiple_of(hn * 8, 8), 8), col * 128:(col + 1) * 128]
            qf = _unpack(_after(yes[0], src, hist[n - RELD])).astype(F32)
            for dd in range(b, b + 4):
                val = jnp.broadcast_to(qf[dd:dd + 1, :], (8, 128))
                qbs[(hh + 1) % 2][dd * 8:(dd + 1) * 8, col * 128:(col + 1) * 128] = val
            return val

        def tied(slot, x):
            for tn, tie in enumerate(ties.get(slot, [])):
                x = _after(yes[tn], x, side_work(tie, slot[1]))
            return x

        for lo, hi in zip(cuts[:-1], cuts[1:]):
            d = stream[lo][0]
            parts = [tied(("k", n), kh_s[d["h"], pl.ds(stream[n][1] * 64 + stream[n][2] * 8, 8), :])
                     for n in range(lo, hi)]
            kk = _unpack(jnp.concatenate(parts, axis=0))[:, 0:DH]
            p = jnp.exp2(_dot(kk, d["qt"]))
            d["l"] = d["l"] + jnp.sum(p.reshape(2 * (hi - lo), 8, TQ), axis=0)
            for n in range(lo, hi):
                _, t, r = stream[n]
                d["grp"][(t, r)] = p[16 * (n - lo):16 * (n - lo) + 16]
                hist[n] = p[16 * (n - lo):16 * (n - lo) + 8, 0:128]
            if hi in pv_at:
                ti = pv_at[hi]
                d, t = tiles[ti]
                if ti != -2:
                    vpu_group(d, t)
                pv_dot(d, t, tied(("v", ti), vt_s[pl.ds(d["r8"], 8), t * CK:(t + 1) * CK]))
                if t == NC - 1:
                    finish(d)

        d = st[-1]
        vpu_group(d, NC - 2)
        for r in range(8):
            carp_s[16 * r:16 * r + 16, :] = d["grp"][(NC - 2, r)]
            if r != POS:
                carp_s[CK + 16 * r:CK + 16 * r + 16, :] = d["grp"][(NC - 1, r)]
        cara_s[0:DH, :] = d["acc"]
        cara_s[DH:DH + 8, :] = d["l"]
        return carry

    lax.fori_loop(0, H // HB, attn_fast, 0)

    dl = carried_unit(H - 1, (H - 1) * 8)
    pv_dot(dl, NC - 2, vt_s[(H - 1) * 8:H * 8, (NC - 2) * CK:(NC - 1) * CK])
    for half in range(2):
        for jj in range(TQ // 128):
            dl["pc"][(NC - 1, half, jj)] = jnp.exp2(vpu_scores(dl, NC - 1, half, jj))
    vpu_group(dl, NC - 1)
    pv_dot(dl, NC - 1, vt_s[(H - 1) * 8:H * 8, (NC - 1) * CK:NC * CK])
    finish(dl)

    def attn_exact(u, carry):
        h = u // NJ
        r8 = pl.multiple_of(h * 8, 8)
        q0 = pl.multiple_of((u % NJ) * TQ, TQ)
        qt = _unpack(qt_s[pl.ds(r8, 8), pl.ds(q0, TQ)])

        def pass1(c, m):
            ku = kh_s[h, pl.ds(pl.multiple_of(c * (CK // 2), CK // 2), CK // 2), :]
            s = _dot(_unpack(ku)[:, 0:DH], qt)
            s_s[pl.ds(pl.multiple_of(c * CK, CK), CK), :] = s
            return jnp.maximum(m, jnp.max(s, axis=0, keepdims=True))

        m = lax.fori_loop(0, NC, pass1, jnp.full((1, TQ), -jnp.inf, F32))

        def pass2(c, la):
            l, acc = la
            c0 = pl.multiple_of(c * CK, CK)
            p = jnp.exp2(s_s[pl.ds(c0, CK), :] - m)
            vt = _unpack(vt_s[pl.ds(r8, 8), pl.ds(c0, CK)])
            return l + jnp.sum(p, axis=0, keepdims=True), acc + _dot(vt, p.astype(BF16))

        l, acc = lax.fori_loop(0, NC, pass2, (jnp.zeros((1, TQ), F32), jnp.zeros((DH, TQ), F32)))
        ot_s[pl.ds(r8, 8), pl.ds(q0, TQ)] = _pack(acc / l)
        return carry

    safe = jnp.logical_and(chk_s[0:1, :] >= L_LO, chk_s[8:9, :] <= L_HI)
    safe = jnp.logical_and(safe, jnp.max(chk_s[16:24, :], axis=0, keepdims=True) <= V_HI)

    @pl.when(jnp.max(jnp.where(safe, 0.0, 1.0)) > 0.0)
    def _():
        lax.fori_loop(0, H * NJ, attn_exact, 0)

    cp_wo.wait()
    cp_win.wait()

    def mix1(r, carry):
        ga = mod_s[0:1, 0:D]
        sb = mod_s[0:1, D:2 * D]
        cb1 = _rb(1.0 + mod_s[0:1, 2 * D:3 * D])

        def stage_a(n):
            r0 = pl.multiple_of(r * TM1 + n * SM1, SM1)
            o = _unpack(ot_s[0:D // 2, pl.ds(r0, SM1)]).astype(F32).T.astype(BF16)
            x1 = x_s[pl.ds(r0, SM1), :].astype(F32) + ga * _dot(o, wo_s[...])
            x1_s[pl.ds(r0, SM1), :] = x1
            return (_ln(x1) * cb1 + sb).astype(BF16)

        def stage_b(n, h2):
            r0 = pl.multiple_of(r * TM1 + n * SM1, SM1)
            r2 = pl.multiple_of(r * (TM1 // 2) + n * (SM1 // 2), SM1 // 2)
            z2_s[pl.ds(r2, SM1 // 2), :] = _pack(_ln(_gelu(_dot(h2, win_s[:, FH:2 * FH]))))
            z1_s[pl.ds(r0, SM1), :] = _gelu(_dot(h2, win_s[:, 0:FH]))

        ns = TM1 // SM1
        h2 = [stage_a(0), stage_a(1)]
        for n in range(ns):
            if n + 2 < ns:
                h2.append(stage_a(n + 2))
            stage_b(n, h2[n])
        return carry

    lax.fori_loop(0, S // TM1, mix1, 0)

    cp_wout.wait()
    cp_wsp.wait()

    def cp_out(t, slot):
        return pltpu.make_async_copy(o_s.at[slot], out_hbm.at[0, pl.ds(t * TM2, TM2), :], sem_out.at[slot])

    def mix2(t, carry):
        slot = t % 2
        gb = mod_s[0:1, 3 * D:4 * D]

        @pl.when(t >= 2)
        def _():
            cp_out(t - 2, slot).wait()

        def gate(n):
            t0 = pl.multiple_of(t * TM2 + n * SM2, SM2)
            g = _dot(wsp_s[pl.ds(t0, SM2), :], _unpack(z2_s[...]))
            b = bcol_s[pl.ds(t0, SM2), :]
            g = g + jnp.concatenate([b] * (FH // 128), axis=1)
            return (z1_s[pl.ds(t0, SM2), :] * g).astype(BF16)

        def proj_out(n, u):
            t0 = pl.multiple_of(t * TM2 + n * SM2, SM2)
            res = x1_s[pl.ds(t0, SM2), :] + gb * _dot(u, wout_s[...])
            o_s[slot, n * SM2:(n + 1) * SM2, :] = res.astype(BF16)

        ns = TM2 // SM2
        u = [gate(n) for n in range(ns)]
        for n in range(ns):
            proj_out(n, u[n])
        cp_out(t, slot).start()
        return carry

    nt = S // TM2
    lax.fori_loop(0, nt, mix2, 0)
    cp_out(nt - 2, (nt - 2) % 2).wait()
    cp_out(nt - 1, (nt - 1) % 2).wait()


@jax.jit
def pallas_adaLN_cond__softmax_full_mha__mixer_gmlp__prompt_kernel(
    A_x: jax.Array,
    A_wqkv: jax.Array,
    A_wo: jax.Array,
    B_x: jax.Array,
    B_w_in: jax.Array,
    B_w_sp: jax.Array,
    B_b_sp: jax.Array,
    B_w_out: jax.Array,
    c: jax.Array,
    w_mod: jax.Array,
):
    del B_x
    hbm = pl.BlockSpec(memory_space=pl.ANY)
    scratch = [
        pltpu.VMEM((S, D), BF16),
        pltpu.VMEM((D, 3 * D), BF16),
        pltpu.VMEM((D, D), BF16),
        pltpu.VMEM((D, 2 * FH), BF16),
        pltpu.VMEM((S, S), BF16),
        pltpu.VMEM((4 * S,), BF16),
        pltpu.VMEM((FH, D), BF16),
        pltpu.VMEM((8, 1, D), BF16),
        pltpu.VMEM((D, 6 * D), BF16),
        pltpu.VMEM((8, 4 * D), F32),
        pltpu.VMEM((8, D), U32),
        pltpu.VMEM((8, S), F32),
        pltpu.VMEM((D, D), U32),
        pltpu.VMEM((S // 2, D), U32),
        pltpu.VMEM((S // 2, D), U32),
        pltpu.VMEM((H, S // 2, 128), U32),
        pltpu.VMEM((D // 2, S), U32),
        pltpu.VMEM((D // 2, S), U32),
        pltpu.VMEM((D // 2 + 8, S), U32),
        pltpu.VMEM((2 * NC, DH * 8, 128), F32),
        pltpu.VMEM((2 * NC, DH * 8, 128), F32),
        pltpu.VMEM((DH * 8, S), F32),
        pltpu.VMEM((DH * 8, S), F32),
        pltpu.VMEM((32, TQ), F32),
        pltpu.VMEM((2 * CK, TQ), F32),
        pltpu.VMEM((32, TQ), F32),
        pltpu.VMEM((S, TQ), F32),
        pltpu.VMEM((S, D), F32),
        pltpu.VMEM((S, FH), F32),
        pltpu.VMEM((S // 2, FH), U32),
        pltpu.VMEM((S, 128), F32),
        pltpu.VMEM((2, TM2, D), BF16),
        pltpu.SemaphoreType.DMA((11,)),
        pltpu.SemaphoreType.DMA((4,)),
        pltpu.SemaphoreType.DMA((4,)),
        pltpu.SemaphoreType.DMA((2,)),
    ]
    return pl.pallas_call(
        _kernel,
        out_shape=jax.ShapeDtypeStruct((1, S, D), BF16),
        in_specs=[hbm] * 9,
        out_specs=hbm,
        scratch_shapes=scratch,
        compiler_params=pltpu.CompilerParams(vmem_limit_bytes=110 * 1024 * 1024),
    )(A_x, A_wqkv, A_wo, B_w_in, B_w_sp, B_b_sp, B_w_out, c, w_mod)
```

```python
import math

import jax
import jax.numpy as jnp
from jax import lax
import jax.experimental.pallas as pl
import jax.experimental.pallas.tpu as pltpu

S = 2048
D = 512
H = 32
DH = 16
FH = 896
EPS = 1e-5

TQ = 512
NJ = S // TQ
CK = 128
NC = S // CK
HB = 2
POS = 0
DELTA = 2
LEAD = 5
CW = 8
QG = 2
GE = 30
RELD = 40
SP = 256
PACE_LO = 0.4
PACE_HI = 0.98
NP2 = 2
TP = 512
TM1 = 512
SM1 = 128
TM2 = 512
SM2 = 128

L_LO = 2.0 ** -30
L_HI = 2.0 ** 60
V_HI = 2.0 ** 60

F32 = jnp.float32
BF16 = jnp.bfloat16
U32 = jnp.uint32


def _ln(x):
    m = jnp.mean(x, axis=-1, keepdims=True)
    xc = x - m
    v = jnp.mean(xc * xc, axis=-1, keepdims=True)
    return xc * lax.rsqrt(v + EPS)


def _gelu(x):
    c = math.sqrt(2.0 / math.pi)
    hx = 0.5 * x
    return hx + hx * jnp.tanh(x * (c + (c * 0.044715) * (x * x)))


def _rb(x):
    return x.astype(BF16).astype(F32)


def _pack(x):
    return pltpu.bitcast(x.astype(BF16), U32)


def _unpack(x):
    return pltpu.bitcast(x, BF16)


def _dot(a, b):
    return jnp.dot(a, b, preferred_element_type=F32)


def _dot_nt(a, b):
    return lax.dot_general(a, b, (((1,), (1,)), ((), ())), preferred_element_type=F32)


def _after(flag, x, dep):
    return jnp.where(flag, x, pltpu.bitcast(dep, U32))


def _paced_dot(flag, lhs, w, deps, lo, hi):
    ng, nn = lhs.shape[0] // 8, w.shape[1] // 128
    at = {}
    for n, row in enumerate(deps):
        idx = int((lo + (hi - lo) * n / max(len(deps) - 1, 1)) * ng * nn)
        at.setdefault(min(idx, ng * nn - 1), []).append(row)
    outs = []
    for j in range(nn):
        col0 = []
        for g in range(ng):
            v = lhs[8 * g:8 * g + 8, 0:128]
            rows = at.get(j * ng + g, [])
            if rows:
                fold = None
                for row in rows:
                    for k in range(row.shape[1] // 128):
                        part = row[:, 128 * k:128 * k + 128]
                        fold = part if fold is None else fold | part
                v = jnp.where(flag, v, fold)
            col0.append(v)
        lj = jnp.concatenate([jnp.concatenate(col0, axis=0), lhs[:, 128:]], axis=1)
        outs.append(_dot(_unpack(lj), w[:, 128 * j:128 * j + 128]))
    return jnp.concatenate(outs, axis=1)


def _row_blocks(x):
    return [x[8 * n:8 * n + 8] for n in range(x.shape[0] // 8)]


def _bcast_k(ku, d):
    return _unpack(jnp.broadcast_to(ku[:, d:d + 1], (8, 128))).astype(F32)


def _kernel(x_hbm, wqkv_hbm, wo_hbm, win_hbm, wsp_hbm, bsp_hbm, wout_hbm, c_hbm, wmod_hbm,
            out_hbm,
            x_s, wqkv_s, wo_s, win_s, wsp_s, bsp_s, wout_s, c_s, wmod_s,
            mod_s, sc_s, brow_s, qvb_s, wqvt_s, h_s, k_s, kh_s, qt_s, vt_s, ot_s, kb0_s, kb1_s, qb0_s, qb1_s, chk_s, carp_s, cara_s, s_s,
            o0_s, x1_s, z1_s, z2_s, bcol_s, o_s,
            sem_in, sem_x, sem_m, sem_out):
    kbs = (kb0_s, kb1_s)
    qbs = (qb0_s, qb1_s)

    def cp_in(src, dst, i):
        return pltpu.make_async_copy(src, dst, sem_in.at[i])

    cp_c = cp_in(c_hbm, c_s.at[0], 0)
    cp_wm1 = cp_in(wmod_hbm.at[:, D:2 * D], wmod_s.at[:, D:2 * D], 1)
    cp_wm0 = cp_in(wmod_hbm.at[:, 0:D], wmod_s.at[:, 0:D], 3)
    cp_wk = cp_in(wqkv_hbm.at[:, D:2 * D], wqkv_s.at[:, D:2 * D], 2)
    cp_wo = cp_in(wo_hbm, wo_s, 4)
    cp_win = cp_in(win_hbm, win_s, 5)
    cp_wsp = cp_in(wsp_hbm, wsp_s, 6)
    cp_bsp = cp_in(bsp_hbm, bsp_s.at[0:S], 7)
    cp_wout = cp_in(wout_hbm, wout_s, 8)
    cp_wq = cp_in(wqkv_hbm.at[:, 0:D], wqkv_s.at[:, 0:D], 9)
    cp_wv = cp_in(wqkv_hbm.at[:, 2 * D:3 * D], wqkv_s.at[:, 2 * D:3 * D], 10)

    xb = (0, 2, 4, 8)

    def cp_x(r):
        rows = pl.ds(xb[r] * SP, (xb[r + 1] - xb[r]) * SP)
        return pltpu.make_async_copy(x_hbm.at[0, rows, :], x_s.at[rows, :], sem_x.at[r])

    def cp_wm2(r):
        cols = pl.ds(pl.multiple_of((2 + r) * D, D), D)
        return pltpu.make_async_copy(wmod_hbm.at[:, cols], wmod_s.at[:, cols], sem_m.at[r])

    cp_c.start()
    cp_wm1.start()
    cp_x(0).start()

    cp_c.wait()
    cp_wk.start()
    cf = c_s[0].astype(F32)
    sc = jnp.broadcast_to((cf * jax.nn.sigmoid(cf)).astype(BF16), (16, D))
    sc_s[...] = pltpu.bitcast(sc, U32)
    cp_x(0).wait()
    n0 = _ln(x_s[0:SP, :].astype(F32))
    cp_wm1.wait()
    cp_x(1).start()
    ca1 = _rb(1.0 + _rb(_dot(sc, wmod_s[:, D:2 * D]))[0:1])

    q_scale = (DH ** -0.5) * math.log2(math.e)
    zsrc0 = pltpu.bitcast(sc, U32)[:, 0:128]
    yes0 = (zsrc0 & 1) <= 1

    def make_h(j, n=None):
        if n is None:
            n = _ln(x_s[j * SP:(j + 1) * SP, :].astype(F32))
        hu = _pack(n * ca1)
        h_s[j * (SP // 2):(j + 1) * (SP // 2), :] = hu
        return hu

    def proj_k(j, hu, dep=None):
        k = _paced_dot(yes0, hu, wqkv_s[:, D:2 * D], _row_blocks(dep), PACE_LO, PACE_HI)
        k_s[j * (SP // 2):(j + 1) * (SP // 2), :] = _pack(k)

    hs = {0: make_h(0, n0)}
    cp_wk.wait()
    cp_x(2).start()
    hs[1] = make_h(1)
    proj_k(0, hs[0], hs[1])
    cp_x(1).wait()
    cp_wm0.start()
    cp_wq.start()
    cp_wv.start()
    hs[2] = make_h(2)
    proj_k(1, hs[1], hs[2])
    hs[3] = make_h(3)
    proj_k(2, hs[2], hs[3])
    cp_x(2).wait()
    for r in range(4):
        cp_wm2(r).start()
    cp_bsp.start()
    hs[4] = make_h(4)
    proj_k(3, hs[3], hs[4])
    hs[5] = make_h(5)
    proj_k(4, hs[4], hs[5])
    hs[6] = make_h(6)
    proj_k(5, hs[5], hs[6])
    cp_wm0.wait()
    cp_wq.wait()
    cp_wv.wait()
    hs[7] = make_h(7)
    wqt = pltpu.bitcast(wqkv_s[:, 0:D].T, U32)
    wvt = pltpu.bitcast(wqkv_s[:, 2 * D:3 * D].T, U32)
    wqvt_s[0:D // 2, :] = wqt
    wqvt_s[D // 2:D, :] = wvt
    proj_k(6, hs[6], jnp.concatenate([hs[7], wqt], axis=0))
    sa = _dot(sc, wmod_s[:, 0:D]).astype(BF16)
    k7a = _paced_dot(yes0, hs[7], wqkv_s[:, D:D + D // 2], _row_blocks(wvt), 0.1, 0.98)
    for part, c0 in enumerate((0, 2 * D)):
        bias = _dot(sa, wqkv_s[:, c0:c0 + D])[0:1]
        for t in range(D // 128):
            qvb_s[part * D + t * 128:part * D + (t + 1) * 128, :] = jnp.broadcast_to(
                bias[:, t * 128:(t + 1) * 128], (128, 128)).T
    k7b = _dot(_unpack(hs[7]), wqkv_s[:, D + D // 2:2 * D])
    k_s[7 * (SP // 2):8 * (SP // 2), :] = _pack(jnp.concatenate([k7a, k7b], axis=1))
    chk_s[0:16, :] = jnp.ones((16, TQ), F32)
    chk_s[16:24, :] = jnp.zeros((8, TQ), F32)
    carp_s[...] = jnp.zeros(carp_s.shape, F32)
    cara_s[...] = jnp.zeros(cara_s.shape, F32)
    kb1_s[2 * NC - 2:2 * NC] = jnp.zeros((2, DH * 8, 128), F32)
    qb1_s[:, S - TQ:S] = jnp.zeros((DH * 8, TQ), F32)
    cp_bsp.wait()
    for cp in (cp_wo, cp_win, cp_wout, cp_wsp):
        cp.start()
    brow_s[...] = jnp.broadcast_to(bsp_s[0:S].reshape(1, S).astype(F32), (8, S))

    def proj_qv_step(r):
        rows = pl.ds(pl.multiple_of(r * (TP // 2), TP // 2), TP // 2)
        cols = pl.ds(pl.multiple_of(r * TP, TP), TP)
        qvt = _dot_nt(_unpack(wqvt_s[...]), _unpack(h_s[rows, :]))
        qvt = qvt + jnp.concatenate([qvb_s[...]] * (TP // 128), axis=1)
        q = (qvt[0:D] * q_scale).astype(BF16)
        qt_s[:, cols] = pltpu.bitcast(q, U32)
        vt_s[:, cols] = _pack(qvt[D:2 * D])
        vmax = jnp.max(jnp.abs(qvt[D:2 * D]).reshape(D // 8, 8, TP), axis=0)
        chk_s[16:24, :] = jnp.maximum(chk_s[16:24, :], vmax)
        q0 = q[0:DH].astype(F32)
        for d in range(DH):
            qb0_s[d * 8:(d + 1) * 8, cols] = jnp.broadcast_to(q0[d:d + 1], (8, TP))
        k = k_s[rows, :]
        for b in range(D // 128):
            kblk = k[:, b * 128:(b + 1) * 128]
            for j in range(8):
                kh_s[b * 8 + j, rows, :] = kblk if j == 0 else pltpu.roll(kblk, 128 - j * DH, 1)
        for t in range(TP // CK):
            ku = k[t * 64 + POS * 8:t * 64 + POS * 8 + 8, 0:128]
            tg = r * (2 * TP // CK) + 2 * t
            for d in range(DH):
                val = _bcast_k(ku, d)
                kb0_s[tg, d * 8:(d + 1) * 8, :] = val[0:8]
                kb0_s[tg + 1, d * 8:(d + 1) * 8, :] = val[8:16]
        mcols = pl.ds(pl.multiple_of((2 + r) * D, D), D)
        mod_s[:, pl.ds(pl.multiple_of(r * D, D), D)] = _rb(_dot(_unpack(sc_s[...]), wmod_s[:, mcols]))[0:8]
        brow = brow_s[0:1, cols]
        for t in range(TP // 128):
            trow = pl.ds(pl.multiple_of(r * TP + t * 128, 128), 128)
            bcol_s[trow, :] = jnp.broadcast_to(brow[:, t * 128:(t + 1) * 128], (128, 128)).T

    def proj_qv(r, carry):
        for n in range(NP2):
            cp_wm2(r * NP2 + n).wait()
        for n in range(NP2):
            proj_qv_step(r * NP2 + n)
        return carry

    lax.fori_loop(0, S // TP // NP2, proj_qv, 0)

    nt_body = HB * NJ * NC

    def vpu_scores(d, t, half, jj):
        c0 = d["q0"] + jj * 128
        m = d["kb"][2 * t + half] * d["qb"][:, c0:c0 + 128]
        return jnp.sum(jnp.sum(m.reshape(DH // 2, 2, 8, 128), axis=0), axis=0)

    def vpu_group(d, t):
        top = jnp.concatenate([d["pc"][(t, 0, jj)] for jj in range(TQ // 128)], axis=1)
        bot = jnp.concatenate([d["pc"][(t, 1, jj)] for jj in range(TQ // 128)], axis=1)
        d["l"] = d["l"] + (top + bot)
        d["grp"][(t, POS)] = jnp.concatenate([top, bot], axis=0)

    def pv_dot(d, t, vt):
        p = jnp.concatenate([d["grp"][(t, r)] for r in range(8)], axis=0)
        d["acc"] = d["acc"] + _dot(_unpack(vt), p.astype(BF16))

    def finish(d):
        l = jnp.sum(d["l"], axis=0, keepdims=True)
        chk_s[0:1, :] = jnp.minimum(chk_s[0:1, :], l)
        chk_s[8:9, :] = jnp.maximum(chk_s[8:9, :], l)
        ot_s[pl.ds(d["o8"], 8), d["q0"]:d["q0"] + TQ] = _pack(d["acc"] * (1.0 / l))

    def carried_unit(h_prev, o8):
        d = dict(r8=pl.multiple_of(h_prev * 8, 8), o8=o8, q0=(NJ - 1) * TQ,
                 kb=kbs[(HB - 1) % 2], qb=qbs[(HB - 1) % 2],
                 acc=cara_s[0:DH, :], l=cara_s[DH:DH + 8, :], grp={}, pc={})
        for r in range(8):
            d["grp"][(NC - 2, r)] = carp_s[16 * r:16 * r + 16, :]
            if r != POS:
                d["grp"][(NC - 1, r)] = carp_s[CK + 16 * r:CK + 16 * r + 16, :]
        return d

    def attn_fast(i, carry):
        zsrc = qt_s[0:8, 0:128]
        yes = [(zsrc & (1 << b)) <= (1 << b) for b in range(4)]
        st = []
        for un in range(HB * NJ):
            h = i * HB + un // NJ
            r8 = pl.multiple_of(h * 8, 8)
            q0 = (un % NJ) * TQ
            st.append(dict(h=h, r8=r8, o8=r8, q0=q0, kb=kbs[(un // NJ) % 2], qb=qbs[(un // NJ) % 2],
                           qt=_unpack(qt_s[pl.ds(r8, 8), q0:q0 + TQ]),
                           acc=jnp.zeros((DH, TQ), F32), l=jnp.zeros((8, TQ), F32),
                           grp={}, pc={}))
        hp = jnp.maximum(i * HB - 1, 0)
        dc = carried_unit(hp, pl.multiple_of(jnp.where(i == 0, H * 8, hp * 8), 8))

        stream, tile_end = [], []
        tiles = {-2: (dc, NC - 2), -1: (dc, NC - 1)}
        for un, d in enumerate(st):
            for t in range(NC):
                stream += [(d, t, r) for r in reversed(range(8)) if r != POS]
                tile_end.append(len(stream))
                tiles[un * NC + t] = (d, t)
        pv_at = {(tile_end[ti + 1] if ti + 1 >= 0 else 0) + DELTA: ti for ti in range(-2, nt_body - 2)}
        slots, slot_of_pv = [], {}
        for n in range(len(stream)):
            if n in pv_at:
                slot_of_pv[pv_at[n]] = len(slots)
                slots.append(("v", pv_at[n]))
            slots.append(("k", n))
        ties = {}
        prev_end = -1
        for ti in range(-1, nt_body - 1):
            end = CW if ti == -1 else slot_of_pv[ti] - LEAD if ti in slot_of_pv else len(slots) - 1
            span = end - prev_end
            for n in range(8):
                pos = prev_end + 1 + (n * span) // 8 if span < 8 else end - ((7 - n) * span) // 8
                ties.setdefault(slots[pos], []).append(("pc", ti, n % 2, n // 2))
            prev_end = end
        per_head = len(stream) // HB
        lo_g, span_g = RELD + 2, per_head - RELD - GE
        kgroups = [(t, b) for b in range(0, DH, 2) for t in range(NC)]
        qgroups = [(col, b) for col in range(S // 128) for b in range(0, DH, QG)]
        for hh in range(HB):
            for n, g in enumerate(kgroups):
                ties.setdefault(("k", hh * per_head + lo_g + (n * span_g) // len(kgroups)), []).append(
                    ("kb", hh) + g)
            for n, g in enumerate(qgroups):
                ties.setdefault(("k", hh * per_head + lo_g + 1 + (n * span_g) // len(qgroups)), []).append(
                    ("qb", hh) + g)
        cuts = set(pv_at) | {0, len(stream)}
        cuts |= {a for a in range(1, len(stream)) if stream[a][0] is not stream[a - 1][0]}
        cuts = sorted(cuts)
        hist = {}

        def side_work(tie, n):
            if tie[0] == "pc":
                _, ti, half, jj = tie
                d, t = tiles[ti]
                s = vpu_scores(d, t, half, jj)
                d["pc"][(t, half, jj)] = jnp.exp2(s)
                return s
            hn = jnp.minimum(i * HB + tie[1] + 1, H - 1)
            if tie[0] == "kb":
                _, hh, tt, b = tie
                src = _after(yes[0], kh_s[hn, pl.ds(tt * 64 + POS * 8, 8), :], hist[n - RELD])
                for dd in range(b, b + 2):
                    val = _bcast_k(src, dd)
                    kbs[(hh + 1) % 2][2 * tt, dd * 8:(dd + 1) * 8, :] = val[0:8]
                    val = val[8:16]
                    kbs[(hh + 1) % 2][2 * tt + 1, dd * 8:(dd + 1) * 8, :] = val
                return val
            _, hh, col, b = tie
            src = qt_s[pl.ds(pl.multiple_of(hn * 8, 8), 8), col * 128:(col + 1) * 128]
            qf = _unpack(_after(yes[0], src, hist[n - RELD])).astype(F32)
            for dd in range(b, b + QG):
                val = jnp.broadcast_to(qf[dd:dd + 1, :], (8, 128))
                qbs[(hh + 1) % 2][dd * 8:(dd + 1) * 8, col * 128:(col + 1) * 128] = val
            return val

        def tied(slot, x):
            for tn, tie in enumerate(ties.get(slot, [])):
                x = _after(yes[tn], x, side_work(tie, slot[1]))
            return x

        for lo, hi in zip(cuts[:-1], cuts[1:]):
            d = stream[lo][0]
            parts = [tied(("k", n), kh_s[d["h"], pl.ds(stream[n][1] * 64 + stream[n][2] * 8, 8), :])
                     for n in range(lo, hi)]
            kk = _unpack(jnp.concatenate(parts, axis=0))[:, 0:DH]
            p = jnp.exp2(_dot(kk, d["qt"]))
            d["l"] = d["l"] + jnp.sum(p.reshape(2 * (hi - lo), 8, TQ), axis=0)
            for n in range(lo, hi):
                _, t, r = stream[n]
                d["grp"][(t, r)] = p[16 * (n - lo):16 * (n - lo) + 16]
                hist[n] = p[16 * (n - lo):16 * (n - lo) + 8, 0:128]
            if hi in pv_at:
                ti = pv_at[hi]
                d, t = tiles[ti]
                if ti != -2:
                    vpu_group(d, t)
                pv_dot(d, t, tied(("v", ti), vt_s[pl.ds(d["r8"], 8), t * CK:(t + 1) * CK]))
                if t == NC - 1:
                    finish(d)

        d = st[-1]
        vpu_group(d, NC - 2)
        for r in range(8):
            carp_s[16 * r:16 * r + 16, :] = d["grp"][(NC - 2, r)]
            if r != POS:
                carp_s[CK + 16 * r:CK + 16 * r + 16, :] = d["grp"][(NC - 1, r)]
        cara_s[0:DH, :] = d["acc"]
        cara_s[DH:DH + 8, :] = d["l"]
        return carry

    lax.fori_loop(0, H // HB, attn_fast, 0)

    dl = carried_unit(H - 1, (H - 1) * 8)
    pv_dot(dl, NC - 2, vt_s[(H - 1) * 8:H * 8, (NC - 2) * CK:(NC - 1) * CK])
    for half in range(2):
        for jj in range(TQ // 128):
            dl["pc"][(NC - 1, half, jj)] = jnp.exp2(vpu_scores(dl, NC - 1, half, jj))
    vpu_group(dl, NC - 1)
    pv_dot(dl, NC - 1, vt_s[(H - 1) * 8:H * 8, (NC - 1) * CK:NC * CK])
    finish(dl)

    def attn_exact(u, carry):
        h = u // NJ
        r8 = pl.multiple_of(h * 8, 8)
        q0 = pl.multiple_of((u % NJ) * TQ, TQ)
        qt = _unpack(qt_s[pl.ds(r8, 8), pl.ds(q0, TQ)])

        def pass1(c, m):
            ku = kh_s[h, pl.ds(pl.multiple_of(c * (CK // 2), CK // 2), CK // 2), :]
            s = _dot(_unpack(ku)[:, 0:DH], qt)
            s_s[pl.ds(pl.multiple_of(c * CK, CK), CK), :] = s
            return jnp.maximum(m, jnp.max(s, axis=0, keepdims=True))

        m = lax.fori_loop(0, NC, pass1, jnp.full((1, TQ), -jnp.inf, F32))

        def pass2(c, la):
            l, acc = la
            c0 = pl.multiple_of(c * CK, CK)
            p = jnp.exp2(s_s[pl.ds(c0, CK), :] - m)
            vt = _unpack(vt_s[pl.ds(r8, 8), pl.ds(c0, CK)])
            return l + jnp.sum(p, axis=0, keepdims=True), acc + _dot(vt, p.astype(BF16))

        l, acc = lax.fori_loop(0, NC, pass2, (jnp.zeros((1, TQ), F32), jnp.zeros((DH, TQ), F32)))
        ot_s[pl.ds(r8, 8), pl.ds(q0, TQ)] = _pack(acc / l)
        return carry

    safe = jnp.logical_and(chk_s[0:1, :] >= L_LO, chk_s[8:9, :] <= L_HI)
    safe = jnp.logical_and(safe, jnp.max(chk_s[16:24, :], axis=0, keepdims=True) <= V_HI)

    @pl.when(jnp.max(jnp.where(safe, 0.0, 1.0)) > 0.0)
    def _():
        lax.fori_loop(0, H * NJ, attn_exact, 0)

    cp_wo.wait()
    cp_win.wait()

    def o_rows(r0):
        return _unpack(ot_s[0:D // 2, pl.ds(r0, SM1)]).astype(F32).T.astype(BF16)

    o0_s[...] = pltpu.bitcast(o_rows(0), U32)

    def mix1(r, carry):
        ga = mod_s[0:1, 0:D]
        sb = mod_s[0:1, D:2 * D]
        cb1 = _rb(1.0 + mod_s[0:1, 2 * D:3 * D])

        def stage_a(n):
            r0 = pl.multiple_of(r * TM1 + n * SM1, SM1)
            o = _unpack(o0_s[...]) if n == 0 else o_rows(r0)
            x1 = x_s[pl.ds(r0, SM1), :].astype(F32) + ga * _dot(o, wo_s[...])
            x1_s[pl.ds(r0, SM1), :] = x1
            return (_ln(x1) * cb1 + sb).astype(BF16)

        def stage_b(n, h2):
            r0 = pl.multiple_of(r * TM1 + n * SM1, SM1)
            r2 = pl.multiple_of(r * (TM1 // 2) + n * (SM1 // 2), SM1 // 2)
            z2_s[pl.ds(r2, SM1 // 2), :] = _pack(_ln(_gelu(_dot(h2, win_s[:, FH:2 * FH]))))
            z1_s[pl.ds(r0, SM1), :] = _gelu(_dot(h2, win_s[:, 0:FH]))

        ns = TM1 // SM1
        h2 = [stage_a(n) for n in range(ns)]
        for n in range(ns):
            stage_b(n, h2[n])
        nxt = pl.multiple_of(jnp.minimum(r + 1, S // TM1 - 1) * TM1, TM1)
        o0_s[...] = pltpu.bitcast(o_rows(nxt), U32)
        return carry

    lax.fori_loop(0, S // TM1, mix1, 0)

    cp_wout.wait()
    cp_wsp.wait()

    def cp_out(j):
        rows = pl.ds(pl.multiple_of(j * SM2, SM2), SM2)
        return pltpu.make_async_copy(o_s.at[rows, :], out_hbm.at[0, rows, :], sem_out.at[0])

    def mix2(t, carry):
        gb = mod_s[0:1, 3 * D:4 * D]

        def gate(n):
            t0 = pl.multiple_of(t * TM2 + n * SM2, SM2)
            g = _dot(wsp_s[pl.ds(t0, SM2), :], _unpack(z2_s[...]))
            b = bcol_s[pl.ds(t0, SM2), :]
            g = g + jnp.concatenate([b] * (FH // 128), axis=1)
            return (z1_s[pl.ds(t0, SM2), :] * g).astype(BF16)

        def proj_out(n, u):
            t0 = pl.multiple_of(t * TM2 + n * SM2, SM2)
            res = x1_s[pl.ds(t0, SM2), :] + gb * _dot(u, wout_s[...])
            o_s[pl.ds(t0, SM2), :] = res.astype(BF16)

        ns = TM2 // SM2
        u = [gate(0)]
        for n in range(ns):
            if n + 1 < ns:
                u.append(gate(n + 1))
            proj_out(n, u[n])
            cp_out(t * ns + n).start()
        return carry

    nt = S // TM2
    lax.fori_loop(0, nt, mix2, 0)
    pltpu.make_async_copy(o_s, out_hbm.at[0], sem_out.at[0]).wait()


@jax.jit
def pallas_adaLN_cond__softmax_full_mha__mixer_gmlp__prompt_kernel(
    A_x: jax.Array,
    A_wqkv: jax.Array,
    A_wo: jax.Array,
    B_x: jax.Array,
    B_w_in: jax.Array,
    B_w_sp: jax.Array,
    B_b_sp: jax.Array,
    B_w_out: jax.Array,
    c: jax.Array,
    w_mod: jax.Array,
):
    del B_x
    hbm = pl.BlockSpec(memory_space=pl.ANY)
    scratch = [
        pltpu.VMEM((S, D), BF16),
        pltpu.VMEM((D, 3 * D), BF16),
        pltpu.VMEM((D, D), BF16),
        pltpu.VMEM((D, 2 * FH), BF16),
        pltpu.VMEM((S, S), BF16),
        pltpu.VMEM((4 * S,), BF16),
        pltpu.VMEM((FH, D), BF16),
        pltpu.VMEM((8, 1, D), BF16),
        pltpu.VMEM((D, 6 * D), BF16),
        pltpu.VMEM((8, 4 * D), F32),
        pltpu.VMEM((8, D), U32),
        pltpu.VMEM((8, S), F32),
        pltpu.VMEM((2 * D, 128), F32),
        pltpu.VMEM((D, D), U32),
        pltpu.VMEM((S // 2, D), U32),
        pltpu.VMEM((S // 2, D), U32),
        pltpu.VMEM((H, S // 2, 128), U32),
        pltpu.VMEM((D // 2, S), U32),
        pltpu.VMEM((D // 2, S), U32),
        pltpu.VMEM((D // 2 + 8, S), U32),
        pltpu.VMEM((2 * NC, DH * 8, 128), F32),
        pltpu.VMEM((2 * NC, DH * 8, 128), F32),
        pltpu.VMEM((DH * 8, S), F32),
        pltpu.VMEM((DH * 8, S), F32),
        pltpu.VMEM((32, TQ), F32),
        pltpu.VMEM((2 * CK, TQ), F32),
        pltpu.VMEM((32, TQ), F32),
        pltpu.VMEM((S, TQ), F32),
        pltpu.VMEM((SM1 // 2, D), U32),
        pltpu.VMEM((S, D), F32),
        pltpu.VMEM((S, FH), F32),
        pltpu.VMEM((S // 2, FH), U32),
        pltpu.VMEM((S, 128), F32),
        pltpu.VMEM((S, D), BF16),
        pltpu.SemaphoreType.DMA((11,)),
        pltpu.SemaphoreType.DMA((4,)),
        pltpu.SemaphoreType.DMA((4,)),
        pltpu.SemaphoreType.DMA((1,)),
    ]
    return pl.pallas_call(
        _kernel,
        out_shape=jax.ShapeDtypeStruct((1, S, D), BF16),
        in_specs=[hbm] * 9,
        out_specs=hbm,
        scratch_shapes=scratch,
        compiler_params=pltpu.CompilerParams(vmem_limit_bytes=110 * 1024 * 1024),
    )(A_x, A_wqkv, A_wo, B_w_in, B_w_sp, B_b_sp, B_w_out, c, w_mod)
```

```python
import math

import jax
import jax.numpy as jnp
from jax import lax
import jax.experimental.pallas as pl
import jax.experimental.pallas.tpu as pltpu

S = 2048
D = 512
H = 32
DH = 16
FH = 896
EPS = 1e-5

TQ = 512
NJ = S // TQ
CK = 128
NC = S // CK
HB = 2
POS = 0
DELTA = 2
LEAD = 5
CW = 8
QG = 2
GE = 30
RELD = 40
SP = 256
PACE_LO = 0.4
PACE_HI = 0.98
NP2 = 2
TP = 512
TM1 = 512
SM1 = 128
TM2 = 512
SM2 = 128

L_LO = 2.0 ** -30
L_HI = 2.0 ** 60
V_HI = 2.0 ** 60

F32 = jnp.float32
BF16 = jnp.bfloat16
U32 = jnp.uint32


def _ln(x):
    m = jnp.mean(x, axis=-1, keepdims=True)
    xc = x - m
    v = jnp.mean(xc * xc, axis=-1, keepdims=True)
    return xc * lax.rsqrt(v + EPS)


def _gelu(x):
    c = math.sqrt(2.0 / math.pi)
    hx = 0.5 * x
    return hx + hx * jnp.tanh(x * (c + (c * 0.044715) * (x * x)))


def _rb(x):
    return x.astype(BF16).astype(F32)


def _pack(x):
    return pltpu.bitcast(x.astype(BF16), U32)


def _unpack(x):
    return pltpu.bitcast(x, BF16)


def _dot(a, b):
    return jnp.dot(a, b, preferred_element_type=F32)


def _dot_nt(a, b):
    return lax.dot_general(a, b, (((1,), (1,)), ((), ())), preferred_element_type=F32)


def _after(flag, x, dep):
    return jnp.where(flag, x, pltpu.bitcast(dep, U32))


def _paced_dot(flag, lhs, w, deps, lo, hi):
    ng, nn = lhs.shape[0] // 8, w.shape[1] // 128
    at = {}
    for n, row in enumerate(deps):
        idx = int((lo + (hi - lo) * n / max(len(deps) - 1, 1)) * ng * nn)
        at.setdefault(min(idx, ng * nn - 1), []).append(row)
    outs = []
    for j in range(nn):
        col0 = []
        for g in range(ng):
            v = lhs[8 * g:8 * g + 8, 0:128]
            rows = at.get(j * ng + g, [])
            if rows:
                fold = None
                for row in rows:
                    for k in range(row.shape[1] // 128):
                        part = row[:, 128 * k:128 * k + 128]
                        fold = part if fold is None else fold | part
                v = jnp.where(flag, v, fold)
            col0.append(v)
        lj = jnp.concatenate([jnp.concatenate(col0, axis=0), lhs[:, 128:]], axis=1)
        outs.append(_dot(_unpack(lj), w[:, 128 * j:128 * j + 128]))
    return jnp.concatenate(outs, axis=1)


def _row_blocks(x):
    return [x[8 * n:8 * n + 8] for n in range(x.shape[0] // 8)]


def _bcast_k(ku, d):
    return _unpack(jnp.broadcast_to(ku[:, d:d + 1], (8, 128))).astype(F32)


def _kernel(x_hbm, wqkv_hbm, wo_hbm, win_hbm, wsp_hbm, bsp_hbm, wout_hbm, c_hbm, wmod_hbm,
            out_hbm,
            x_s, wqkv_s, wo_s, win_s, wsp_s, bsp_s, wout_s, c_s, wmod_s,
            mod_s, sc_s, brow_s, qvb_s, wqvt_s, h_s, k_s, kh_s, qt_s, vt_s, ot_s,
            kb0_s, kb1_s, qb0_s, qb1_s, chk_s, carp_s, cara_s, s_s,
            o0_s, x1_s, z1_s, z2_s, bcol_s, o_s,
            sem_in, sem_x, sem_m, sem_out):
    kbs = (kb0_s, kb1_s)
    qbs = (qb0_s, qb1_s)

    def cp_in(src, dst, i):
        return pltpu.make_async_copy(src, dst, sem_in.at[i])

    cp_c = cp_in(c_hbm, c_s.at[0], 0)
    cp_wm1 = cp_in(wmod_hbm.at[:, D:2 * D], wmod_s.at[:, D:2 * D], 1)
    cp_wm0 = cp_in(wmod_hbm.at[:, 0:D], wmod_s.at[:, 0:D], 3)
    cp_wk = cp_in(wqkv_hbm.at[:, D:2 * D], wqkv_s.at[:, D:2 * D], 2)
    cp_wo = cp_in(wo_hbm, wo_s, 4)
    cp_win = cp_in(win_hbm, win_s, 5)
    cp_wsp = cp_in(wsp_hbm, wsp_s, 6)
    cp_bsp = cp_in(bsp_hbm, bsp_s.at[0:S], 7)
    cp_wout = cp_in(wout_hbm, wout_s, 8)
    cp_wq = cp_in(wqkv_hbm.at[:, 0:D], wqkv_s.at[:, 0:D], 9)
    cp_wv = cp_in(wqkv_hbm.at[:, 2 * D:3 * D], wqkv_s.at[:, 2 * D:3 * D], 10)

    xb = (0, 2, 4, 8)

    def cp_x(r):
        rows = pl.ds(xb[r] * SP, (xb[r + 1] - xb[r]) * SP)
        return pltpu.make_async_copy(x_hbm.at[0, rows, :], x_s.at[rows, :], sem_x.at[r])

    def cp_wm2(r):
        cols = pl.ds(pl.multiple_of((2 + r) * D, D), D)
        return pltpu.make_async_copy(wmod_hbm.at[:, cols], wmod_s.at[:, cols], sem_m.at[r])

    cp_c.start()
    cp_x(0).start()
    cp_wm1.start()

    cp_c.wait()
    cp_wk.start()
    cf = c_s[0].astype(F32)
    sc = jnp.broadcast_to((cf * jax.nn.sigmoid(cf)).astype(BF16), (16, D))
    sc_s[...] = pltpu.bitcast(sc, U32)
    cp_x(0).wait()
    n0 = _ln(x_s[0:SP, :].astype(F32))
    cp_wm1.wait()
    cp_x(1).start()
    ca1 = _rb(1.0 + _rb(_dot(sc, wmod_s[:, D:2 * D]))[0:1])

    q_scale = (DH ** -0.5) * math.log2(math.e)
    zsrc0 = pltpu.bitcast(sc, U32)[:, 0:128]
    yes0 = (zsrc0 & 1) <= 1

    def make_h(j, n=None):
        if n is None:
            n = _ln(x_s[j * SP:(j + 1) * SP, :].astype(F32))
        hu = _pack(n * ca1)
        h_s[j * (SP // 2):(j + 1) * (SP // 2), :] = hu
        return hu

    def proj_k(j, hu, dep):
        k = _paced_dot(yes0, hu, wqkv_s[:, D:2 * D], _row_blocks(dep), PACE_LO, PACE_HI)
        k_s[j * (SP // 2):(j + 1) * (SP // 2), :] = _pack(k)

    hs = {0: make_h(0, n0)}
    cp_wk.wait()
    cp_x(2).start()
    hs[1] = make_h(1)
    proj_k(0, hs[0], hs[1])
    cp_x(1).wait()
    cp_bsp.start()
    cp_wm0.start()
    cp_wq.start()
    cp_wv.start()
    hs[2] = make_h(2)
    proj_k(1, hs[1], hs[2])
    hs[3] = make_h(3)
    proj_k(2, hs[2], hs[3])
    cp_x(2).wait()
    for r in range(4):
        cp_wm2(r).start()
    hs[4] = make_h(4)
    proj_k(3, hs[3], hs[4])
    hs[5] = make_h(5)
    proj_k(4, hs[4], hs[5])
    hs[6] = make_h(6)
    proj_k(5, hs[5], hs[6])
    cp_wm0.wait()
    cp_wq.wait()
    cp_wv.wait()
    cp_bsp.wait()
    brow_s[...] = jnp.broadcast_to(bsp_s[0:S].reshape(1, S).astype(F32), (8, S))
    hs[7] = make_h(7)
    wqt = pltpu.bitcast(wqkv_s[:, 0:D].T, U32)
    wvt = pltpu.bitcast(wqkv_s[:, 2 * D:3 * D].T, U32)
    wqvt_s[0:D // 2, :] = wqt
    wqvt_s[D // 2:D, :] = wvt
    proj_k(6, hs[6], jnp.concatenate([hs[7], wqt], axis=0))
    sa = _dot(sc, wmod_s[:, 0:D]).astype(BF16)
    k7a = _paced_dot(yes0, hs[7], wqkv_s[:, D:D + D // 2], _row_blocks(wvt), 0.1, 0.98)
    for part, c0 in enumerate((0, 2 * D)):
        bias = _dot(sa, wqkv_s[:, c0:c0 + D])[0:1]
        for t in range(D // 128):
            qvb_s[part * D + t * 128:part * D + (t + 1) * 128, :] = jnp.broadcast_to(
                bias[:, t * 128:(t + 1) * 128], (128, 128)).T
    k7b = _dot(_unpack(hs[7]), wqkv_s[:, D + D // 2:2 * D])
    k_s[7 * (SP // 2):8 * (SP // 2), :] = _pack(jnp.concatenate([k7a, k7b], axis=1))
    chk_s[0:16, :] = jnp.ones((16, TQ), F32)
    chk_s[16:24, :] = jnp.zeros((8, TQ), F32)
    carp_s[...] = jnp.zeros(carp_s.shape, F32)
    cara_s[...] = jnp.zeros(cara_s.shape, F32)
    kb1_s[2 * NC - 2:2 * NC] = jnp.zeros((2, DH * 8, 128), F32)
    qb1_s[:, S - TQ:S] = jnp.zeros((DH * 8, TQ), F32)
    for cp in (cp_wo, cp_win, cp_wout, cp_wsp):
        cp.start()

    def proj_qv_step(r):
        rows = pl.ds(pl.multiple_of(r * (TP // 2), TP // 2), TP // 2)
        cols = pl.ds(pl.multiple_of(r * TP, TP), TP)
        qvt = _dot_nt(_unpack(wqvt_s[...]), _unpack(h_s[rows, :]))
        qvt = qvt + jnp.concatenate([qvb_s[...]] * (TP // 128), axis=1)
        q = (qvt[0:D] * q_scale).astype(BF16)
        qt_s[:, cols] = pltpu.bitcast(q, U32)
        vt_s[:, cols] = _pack(qvt[D:2 * D])
        vmax = jnp.max(jnp.abs(qvt[D:2 * D]).reshape(D // 8, 8, TP), axis=0)
        chk_s[16:24, :] = jnp.maximum(chk_s[16:24, :], vmax)
        q0 = q[0:DH].astype(F32)
        for d in range(DH):
            qb0_s[d * 8:(d + 1) * 8, cols] = jnp.broadcast_to(q0[d:d + 1], (8, TP))
        k = k_s[rows, :]
        for b in range(D // 128):
            kblk = k[:, b * 128:(b + 1) * 128]
            for j in range(8):
                kh_s[b * 8 + j, rows, :] = kblk if j == 0 else pltpu.roll(kblk, 128 - j * DH, 1)
        for t in range(TP // CK):
            ku = k[t * 64 + POS * 8:t * 64 + POS * 8 + 8, 0:128]
            tg = r * (2 * TP // CK) + 2 * t
            for d in range(DH):
                val = _bcast_k(ku, d)
                kb0_s[tg, d * 8:(d + 1) * 8, :] = val[0:8]
                kb0_s[tg + 1, d * 8:(d + 1) * 8, :] = val[8:16]
        mcols = pl.ds(pl.multiple_of((2 + r) * D, D), D)
        mod_s[:, pl.ds(pl.multiple_of(r * D, D), D)] = _rb(_dot(_unpack(sc_s[...]), wmod_s[:, mcols]))[0:8]
        brow = brow_s[0:1, cols]
        for t in range(TP // 128):
            trow = pl.ds(pl.multiple_of(r * TP + t * 128, 128), 128)
            bcol_s[trow, :] = jnp.broadcast_to(brow[:, t * 128:(t + 1) * 128], (128, 128)).T

    def proj_qv(r, carry):
        for n in range(NP2):
            cp_wm2(r * NP2 + n).wait()
        for n in range(NP2):
            proj_qv_step(r * NP2 + n)
        return carry

    lax.fori_loop(0, S // TP // NP2, proj_qv, 0)

    nt_body = HB * NJ * NC

    def vpu_scores(d, t, half, jj):
        c0 = d["q0"] + jj * 128
        m = d["kb"][2 * t + half] * d["qb"][:, c0:c0 + 128]
        return jnp.sum(jnp.sum(m.reshape(DH // 2, 2, 8, 128), axis=0), axis=0)

    def vpu_group(d, t):
        top = jnp.concatenate([d["pc"][(t, 0, jj)] for jj in range(TQ // 128)], axis=1)
        bot = jnp.concatenate([d["pc"][(t, 1, jj)] for jj in range(TQ // 128)], axis=1)
        d["l"] = d["l"] + (top + bot)
        d["grp"][(t, POS)] = jnp.concatenate([top, bot], axis=0)

    def pv_dot(d, t, vt):
        p = jnp.concatenate([d["grp"][(t, r)] for r in range(8)], axis=0)
        d["acc"] = d["acc"] + _dot(_unpack(vt), p.astype(BF16))

    def finish(d):
        l = jnp.sum(d["l"], axis=0, keepdims=True)
        chk_s[0:1, :] = jnp.minimum(chk_s[0:1, :], l)
        chk_s[8:9, :] = jnp.maximum(chk_s[8:9, :], l)
        ot_s[pl.ds(d["o8"], 8), d["q0"]:d["q0"] + TQ] = _pack(d["acc"] * (1.0 / l))

    def carried_unit(h_prev, o8):
        d = dict(r8=pl.multiple_of(h_prev * 8, 8), o8=o8, q0=(NJ - 1) * TQ,
                 kb=kbs[(HB - 1) % 2], qb=qbs[(HB - 1) % 2],
                 acc=cara_s[0:DH, :], l=cara_s[DH:DH + 8, :], grp={}, pc={})
        for r in range(8):
            d["grp"][(NC - 2, r)] = carp_s[16 * r:16 * r + 16, :]
            if r != POS:
                d["grp"][(NC - 1, r)] = carp_s[CK + 16 * r:CK + 16 * r + 16, :]
        return d

    def attn_fast(i, carry):
        zsrc = qt_s[0:8, 0:128]
        yes = [(zsrc & (1 << b)) <= (1 << b) for b in range(4)]
        st = []
        for un in range(HB * NJ):
            h = i * HB + un // NJ
            r8 = pl.multiple_of(h * 8, 8)
            q0 = (un % NJ) * TQ
            st.append(dict(h=h, r8=r8, o8=r8, q0=q0, kb=kbs[(un // NJ) % 2], qb=qbs[(un // NJ) % 2],
                           qt=_unpack(qt_s[pl.ds(r8, 8), q0:q0 + TQ]),
                           acc=jnp.zeros((DH, TQ), F32), l=jnp.zeros((8, TQ), F32),
                           grp={}, pc={}))
        hp = jnp.maximum(i * HB - 1, 0)
        dc = carried_unit(hp, pl.multiple_of(jnp.where(i == 0, H * 8, hp * 8), 8))

        stream, tile_end = [], []
        tiles = {-2: (dc, NC - 2), -1: (dc, NC - 1)}
        for un, d in enumerate(st):
            for t in range(NC):
                stream += [(d, t, r) for r in reversed(range(8)) if r != POS]
                tile_end.append(len(stream))
                tiles[un * NC + t] = (d, t)
        pv_at = {(tile_end[ti + 1] if ti + 1 >= 0 else 0) + DELTA: ti for ti in range(-2, nt_body - 2)}
        slots, slot_of_pv = [], {}
        for n in range(len(stream)):
            if n in pv_at:
                slot_of_pv[pv_at[n]] = len(slots)
                slots.append(("v", pv_at[n]))
            slots.append(("k", n))
        ties = {}
        prev_end = -1
        for ti in range(-1, nt_body - 1):
            end = CW if ti == -1 else slot_of_pv[ti] - LEAD if ti in slot_of_pv else len(slots) - 1
            span = end - prev_end
            for n in range(8):
                pos = prev_end + 1 + (n * span) // 8 if span < 8 else end - ((7 - n) * span) // 8
                ties.setdefault(slots[pos], []).append(("pc", ti, n % 2, n // 2))
            prev_end = end
        per_head = len(stream) // HB
        lo_g, span_g = RELD + 2, per_head - RELD - GE
        kgroups = [(t, b) for b in range(0, DH, 2) for t in range(NC)]
        qgroups = [(col, b) for col in range(S // 128) for b in range(0, DH, QG)]
        for hh in range(HB):
            for n, g in enumerate(kgroups):
                ties.setdefault(("k", hh * per_head + lo_g + (n * span_g) // len(kgroups)), []).append(
                    ("kb", hh) + g)
            for n, g in enumerate(qgroups):
                ties.setdefault(("k", hh * per_head + lo_g + 1 + (n * span_g) // len(qgroups)), []).append(
                    ("qb", hh) + g)
        cuts = set(pv_at) | {0, len(stream)}
        cuts |= {a for a in range(1, len(stream)) if stream[a][0] is not stream[a - 1][0]}
        cuts = sorted(cuts)
        hist = {}

        def side_work(tie, n):
            if tie[0] == "pc":
                _, ti, half, jj = tie
                d, t = tiles[ti]
                s = vpu_scores(d, t, half, jj)
                d["pc"][(t, half, jj)] = jnp.exp2(s)
                return s
            hn = jnp.minimum(i * HB + tie[1] + 1, H - 1)
            if tie[0] == "kb":
                _, hh, tt, b = tie
                src = _after(yes[0], kh_s[hn, pl.ds(tt * 64 + POS * 8, 8), :], hist[n - RELD])
                for dd in range(b, b + 2):
                    val = _bcast_k(src, dd)
                    kbs[(hh + 1) % 2][2 * tt, dd * 8:(dd + 1) * 8, :] = val[0:8]
                    val = val[8:16]
                    kbs[(hh + 1) % 2][2 * tt + 1, dd * 8:(dd + 1) * 8, :] = val
                return val
            _, hh, col, b = tie
            src = qt_s[pl.ds(pl.multiple_of(hn * 8, 8), 8), col * 128:(col + 1) * 128]
            qf = _unpack(_after(yes[0], src, hist[n - RELD])).astype(F32)
            for dd in range(b, b + QG):
                val = jnp.broadcast_to(qf[dd:dd + 1, :], (8, 128))
                qbs[(hh + 1) % 2][dd * 8:(dd + 1) * 8, col * 128:(col + 1) * 128] = val
            return val

        def tied(slot, x):
            for tn, tie in enumerate(ties.get(slot, [])):
                x = _after(yes[tn], x, side_work(tie, slot[1]))
            return x

        for lo, hi in zip(cuts[:-1], cuts[1:]):
            d = stream[lo][0]
            parts = [tied(("k", n), kh_s[d["h"], pl.ds(stream[n][1] * 64 + stream[n][2] * 8, 8), :])
                     for n in range(lo, hi)]
            kk = _unpack(jnp.concatenate(parts, axis=0))[:, 0:DH]
            p = jnp.exp2(_dot(kk, d["qt"]))
            d["l"] = d["l"] + jnp.sum(p.reshape(2 * (hi - lo), 8, TQ), axis=0)
            for n in range(lo, hi):
                _, t, r = stream[n]
                d["grp"][(t, r)] = p[16 * (n - lo):16 * (n - lo) + 16]
                hist[n] = p[16 * (n - lo):16 * (n - lo) + 8, 0:128]
            if hi in pv_at:
                ti = pv_at[hi]
                d, t = tiles[ti]
                if ti != -2:
                    vpu_group(d, t)
                pv_dot(d, t, tied(("v", ti), vt_s[pl.ds(d["r8"], 8), t * CK:(t + 1) * CK]))
                if t == NC - 1:
                    finish(d)

        d = st[-1]
        vpu_group(d, NC - 2)
        for r in range(8):
            carp_s[16 * r:16 * r + 16, :] = d["grp"][(NC - 2, r)]
            if r != POS:
                carp_s[CK + 16 * r:CK + 16 * r + 16, :] = d["grp"][(NC - 1, r)]
        cara_s[0:DH, :] = d["acc"]
        cara_s[DH:DH + 8, :] = d["l"]
        return carry

    lax.fori_loop(0, H // HB, attn_fast, 0)

    def o_rows(r0):
        return _unpack(ot_s[0:D // 2, pl.ds(r0, SM1)]).astype(F32).T.astype(BF16)

    o0_s[...] = pltpu.bitcast(o_rows(0), U32)

    dl = carried_unit(H - 1, (H - 1) * 8)
    pv_dot(dl, NC - 2, vt_s[(H - 1) * 8:H * 8, (NC - 2) * CK:(NC - 1) * CK])
    for half in range(2):
        for jj in range(TQ // 128):
            dl["pc"][(NC - 1, half, jj)] = jnp.exp2(vpu_scores(dl, NC - 1, half, jj))
    vpu_group(dl, NC - 1)
    pv_dot(dl, NC - 1, vt_s[(H - 1) * 8:H * 8, (NC - 1) * CK:NC * CK])
    finish(dl)

    def attn_exact(u, carry):
        h = u // NJ
        r8 = pl.multiple_of(h * 8, 8)
        q0 = pl.multiple_of((u % NJ) * TQ, TQ)
        qt = _unpack(qt_s[pl.ds(r8, 8), pl.ds(q0, TQ)])

        def pass1(c, m):
            ku = kh_s[h, pl.ds(pl.multiple_of(c * (CK // 2), CK // 2), CK // 2), :]
            s = _dot(_unpack(ku)[:, 0:DH], qt)
            s_s[pl.ds(pl.multiple_of(c * CK, CK), CK), :] = s
            return jnp.maximum(m, jnp.max(s, axis=0, keepdims=True))

        m = lax.fori_loop(0, NC, pass1, jnp.full((1, TQ), -jnp.inf, F32))

        def pass2(c, la):
            l, acc = la
            c0 = pl.multiple_of(c * CK, CK)
            p = jnp.exp2(s_s[pl.ds(c0, CK), :] - m)
            vt = _unpack(vt_s[pl.ds(r8, 8), pl.ds(c0, CK)])
            return l + jnp.sum(p, axis=0, keepdims=True), acc + _dot(vt, p.astype(BF16))

        l, acc = lax.fori_loop(0, NC, pass2, (jnp.zeros((1, TQ), F32), jnp.zeros((DH, TQ), F32)))
        ot_s[pl.ds(r8, 8), pl.ds(q0, TQ)] = _pack(acc / l)
        return carry

    safe = jnp.logical_and(chk_s[0:1, :] >= L_LO, chk_s[8:9, :] <= L_HI)
    safe = jnp.logical_and(safe, jnp.max(chk_s[16:24, :], axis=0, keepdims=True) <= V_HI)

    @pl.when(jnp.max(jnp.where(safe, 0.0, 1.0)) > 0.0)
    def _():
        lax.fori_loop(0, H * NJ, attn_exact, 0)
        o0_s[...] = pltpu.bitcast(o_rows(0), U32)

    cp_wo.wait()
    cp_win.wait()

    def mix1(r, carry):
        ga = mod_s[0:1, 0:D]
        sb = mod_s[0:1, D:2 * D]
        cb1 = _rb(1.0 + mod_s[0:1, 2 * D:3 * D])

        def stage_a(n):
            r0 = pl.multiple_of(r * TM1 + n * SM1, SM1)
            o = _unpack(o0_s[...]) if n == 0 else o_rows(r0)
            x1 = x_s[pl.ds(r0, SM1), :].astype(F32) + ga * _dot(o, wo_s[...])
            x1_s[pl.ds(r0, SM1), :] = x1
            return (_ln(x1) * cb1 + sb).astype(BF16)

        def stage_b(n, h2):
            r0 = pl.multiple_of(r * TM1 + n * SM1, SM1)
            r2 = pl.multiple_of(r * (TM1 // 2) + n * (SM1 // 2), SM1 // 2)
            z2_s[pl.ds(r2, SM1 // 2), :] = _pack(_ln(_gelu(_dot(h2, win_s[:, FH:2 * FH]))))
            z1_s[pl.ds(r0, SM1), :] = _gelu(_dot(h2, win_s[:, 0:FH]))

        ns = TM1 // SM1
        h2 = [stage_a(n) for n in range(ns)]
        for n in range(ns):
            stage_b(n, h2[n])
        nxt = pl.multiple_of(jnp.minimum(r + 1, S // TM1 - 1) * TM1, TM1)
        o0_s[...] = pltpu.bitcast(o_rows(nxt), U32)
        return carry

    lax.fori_loop(0, S // TM1, mix1, 0)

    cp_wout.wait()
    cp_wsp.wait()

    def cp_out(j):
        rows = pl.ds(pl.multiple_of(j * SM2, SM2), SM2)
        return pltpu.make_async_copy(o_s.at[rows, :], out_hbm.at[0, rows, :], sem_out.at[0])

    def mix2(t, carry):
        gb = mod_s[0:1, 3 * D:4 * D]

        def gate(n):
            t0 = pl.multiple_of(t * TM2 + n * SM2, SM2)
            g = _dot(wsp_s[pl.ds(t0, SM2), :], _unpack(z2_s[...]))
            b = bcol_s[pl.ds(t0, SM2), :]
            g = g + jnp.concatenate([b] * (FH // 128), axis=1)
            return (z1_s[pl.ds(t0, SM2), :] * g).astype(BF16)

        def proj_out(n, u):
            t0 = pl.multiple_of(t * TM2 + n * SM2, SM2)
            res = x1_s[pl.ds(t0, SM2), :] + gb * _dot(u, wout_s[...])
            o_s[pl.ds(t0, SM2), :] = res.astype(BF16)

        ns = TM2 // SM2
        u = [gate(0)]
        for n in range(ns):
            if n + 1 < ns:
                u.append(gate(n + 1))
            proj_out(n, u[n])
            cp_out(t * ns + n).start()
        return carry

    nt = S // TM2
    lax.fori_loop(0, nt, mix2, 0)
    pltpu.make_async_copy(o_s, out_hbm.at[0], sem_out.at[0]).wait()


@jax.jit
def pallas_adaLN_cond__softmax_full_mha__mixer_gmlp__prompt_kernel(
    A_x: jax.Array,
    A_wqkv: jax.Array,
    A_wo: jax.Array,
    B_x: jax.Array,
    B_w_in: jax.Array,
    B_w_sp: jax.Array,
    B_b_sp: jax.Array,
    B_w_out: jax.Array,
    c: jax.Array,
    w_mod: jax.Array,
):
    del B_x
    hbm = pl.BlockSpec(memory_space=pl.ANY)
    scratch = [
        pltpu.VMEM((S, D), BF16),
        pltpu.VMEM((D, 3 * D), BF16),
        pltpu.VMEM((D, D), BF16),
        pltpu.VMEM((D, 2 * FH), BF16),
        pltpu.VMEM((S, S), BF16),
        pltpu.VMEM((4 * S,), BF16),
        pltpu.VMEM((FH, D), BF16),
        pltpu.VMEM((8, 1, D), BF16),
        pltpu.VMEM((D, 6 * D), BF16),
        pltpu.VMEM((8, 4 * D), F32),
        pltpu.VMEM((8, D), U32),
        pltpu.VMEM((8, S), F32),
        pltpu.VMEM((2 * D, 128), F32),
        pltpu.VMEM((D, D), U32),
        pltpu.VMEM((S // 2, D), U32),
        pltpu.VMEM((S // 2, D), U32),
        pltpu.VMEM((H, S // 2, 128), U32),
        pltpu.VMEM((D // 2, S), U32),
        pltpu.VMEM((D // 2, S), U32),
        pltpu.VMEM((D // 2 + 8, S), U32),
        pltpu.VMEM((2 * NC, DH * 8, 128), F32),
        pltpu.VMEM((2 * NC, DH * 8, 128), F32),
        pltpu.VMEM((DH * 8, S), F32),
        pltpu.VMEM((DH * 8, S), F32),
        pltpu.VMEM((32, TQ), F32),
        pltpu.VMEM((2 * CK, TQ), F32),
        pltpu.VMEM((32, TQ), F32),
        pltpu.VMEM((S, TQ), F32),
        pltpu.VMEM((SM1 // 2, D), U32),
        pltpu.VMEM((S, D), F32),
        pltpu.VMEM((S, FH), F32),
        pltpu.VMEM((S // 2, FH), U32),
        pltpu.VMEM((S, 128), F32),
        pltpu.VMEM((S, D), BF16),
        pltpu.SemaphoreType.DMA((11,)),
        pltpu.SemaphoreType.DMA((3,)),
        pltpu.SemaphoreType.DMA((4,)),
        pltpu.SemaphoreType.DMA((1,)),
    ]
    return pl.pallas_call(
        _kernel,
        out_shape=jax.ShapeDtypeStruct((1, S, D), BF16),
        in_specs=[hbm] * 9,
        out_specs=hbm,
        scratch_shapes=scratch,
        compiler_params=pltpu.CompilerParams(vmem_limit_bytes=110 * 1024 * 1024),
    )(A_x, A_wqkv, A_wo, B_w_in, B_w_sp, B_b_sp, B_w_out, c, w_mod)
```

```python
import math

import jax
import jax.numpy as jnp
from jax import lax
import jax.experimental.pallas as pl
import jax.experimental.pallas.tpu as pltpu

S = 2048
D = 512
H = 32
DH = 16
FH = 896
EPS = 1e-5

TQ = 512
NJ = S // TQ
CK = 128
NC = S // CK
HB = 2
POS = 0
SKIP = (1, 6, 11)
DELTA = 2
LEAD = 5
CW = 8
QG = 2
GE = 30
RELD = 41
SP = 256
PACE_LO = 0.4
PACE_HI = 0.98
NP2 = 2
TP = 512
TM1 = 512
SM1 = 128
TM2 = 512
SM2 = 128

L_LO = 2.0 ** -30
L_HI = 2.0 ** 60
V_HI = 2.0 ** 60

F32 = jnp.float32
BF16 = jnp.bfloat16
U32 = jnp.uint32


def _ln(x):
    m = jnp.mean(x, axis=-1, keepdims=True)
    xc = x - m
    v = jnp.mean(xc * xc, axis=-1, keepdims=True)
    return xc * lax.rsqrt(v + EPS)


def _gelu(x):
    c = math.sqrt(2.0 / math.pi)
    hx = 0.5 * x
    return hx + hx * jnp.tanh(x * (c + (c * 0.044715) * (x * x)))


def _rb(x):
    return x.astype(BF16).astype(F32)


def _pack(x):
    return pltpu.bitcast(x.astype(BF16), U32)


def _unpack(x):
    return pltpu.bitcast(x, BF16)


def _dot(a, b):
    return jnp.dot(a, b, preferred_element_type=F32)


def _dot_nt(a, b):
    return lax.dot_general(a, b, (((1,), (1,)), ((), ())), preferred_element_type=F32)


def _after(flag, x, dep):
    return jnp.where(flag, x, pltpu.bitcast(dep, U32))


def _paced_dot(flag, lhs, w, deps, lo, hi):
    ng, nn = lhs.shape[0] // 8, w.shape[1] // 128
    at = {}
    for n, row in enumerate(deps):
        idx = int((lo + (hi - lo) * n / max(len(deps) - 1, 1)) * ng * nn)
        at.setdefault(min(idx, ng * nn - 1), []).append(row)
    outs = []
    for j in range(nn):
        col0 = []
        for g in range(ng):
            v = lhs[8 * g:8 * g + 8, 0:128]
            rows = at.get(j * ng + g, [])
            if rows:
                fold = None
                for row in rows:
                    for k in range(row.shape[1] // 128):
                        part = row[:, 128 * k:128 * k + 128]
                        fold = part if fold is None else fold | part
                v = jnp.where(flag, v, fold)
            col0.append(v)
        lj = jnp.concatenate([jnp.concatenate(col0, axis=0), lhs[:, 128:]], axis=1)
        outs.append(_dot(_unpack(lj), w[:, 128 * j:128 * j + 128]))
    return jnp.concatenate(outs, axis=1)


def _row_blocks(x):
    return [x[8 * n:8 * n + 8] for n in range(x.shape[0] // 8)]


def _bcast_k(ku, d):
    return _unpack(jnp.broadcast_to(ku[:, d:d + 1], (8, 128))).astype(F32)


def _kernel(x_hbm, wqkv_hbm, wo_hbm, win_hbm, wsp_hbm, bsp_hbm, wout_hbm, c_hbm, wmod_hbm,
            out_hbm,
            x_s, wqkv_s, wo_s, win_s, wsp_s, bsp_s, wout_s, c_s, wmod_s,
            mod_s, sc_s, brow_s, qvb_s, wqvt_s, h_s, k_s, kh_s, qt_s, vt_s, ot_s,
            kb0_s, kb1_s, qb0_s, qb1_s, chk_s, carp_s, cara_s, s_s,
            o0_s, x1_s, z1_s, z2_s, bcol_s, o_s,
            sem_in, sem_x, sem_m, sem_out):
    kbs = (kb0_s, kb1_s)
    qbs = (qb0_s, qb1_s)

    def cp_in(src, dst, i):
        return pltpu.make_async_copy(src, dst, sem_in.at[i])

    cp_c = cp_in(c_hbm, c_s.at[0], 0)
    cp_wm1 = cp_in(wmod_hbm.at[:, D:2 * D], wmod_s.at[:, D:2 * D], 1)
    cp_wm0 = cp_in(wmod_hbm.at[:, 0:D], wmod_s.at[:, 0:D], 3)
    cp_wk = cp_in(wqkv_hbm.at[:, D:2 * D], wqkv_s.at[:, D:2 * D], 2)
    cp_wo = cp_in(wo_hbm, wo_s, 4)
    cp_win = cp_in(win_hbm, win_s, 5)
    cp_wsp = cp_in(wsp_hbm, wsp_s, 6)
    cp_bsp = cp_in(bsp_hbm, bsp_s.at[0:S], 7)
    cp_wout = cp_in(wout_hbm, wout_s, 8)
    cp_wq = cp_in(wqkv_hbm.at[:, 0:D], wqkv_s.at[:, 0:D], 9)
    cp_wv = cp_in(wqkv_hbm.at[:, 2 * D:3 * D], wqkv_s.at[:, 2 * D:3 * D], 10)

    xb = (0, 2, 4, 8)

    def cp_x(r):
        rows = pl.ds(xb[r] * SP, (xb[r + 1] - xb[r]) * SP)
        return pltpu.make_async_copy(x_hbm.at[0, rows, :], x_s.at[rows, :], sem_x.at[r])

    def cp_wm2(r):
        cols = pl.ds(pl.multiple_of((2 + r) * D, D), D)
        return pltpu.make_async_copy(wmod_hbm.at[:, cols], wmod_s.at[:, cols], sem_m.at[r])

    cp_c.start()
    cp_x(0).start()
    cp_wm1.start()

    cp_c.wait()
    cp_wk.start()
    cf = c_s[0].astype(F32)
    sc = jnp.broadcast_to((cf * jax.nn.sigmoid(cf)).astype(BF16), (16, D))
    sc_s[...] = pltpu.bitcast(sc, U32)
    cp_x(0).wait()
    n0 = _ln(x_s[0:SP, :].astype(F32))
    cp_wm1.wait()
    cp_x(1).start()
    ca1 = _rb(1.0 + _rb(_dot(sc, wmod_s[:, D:2 * D]))[0:1])

    q_scale = (DH ** -0.5) * math.log2(math.e)
    zsrc0 = pltpu.bitcast(sc, U32)[:, 0:128]
    yes0 = (zsrc0 & 1) <= 1

    def make_h(j, n=None):
        if n is None:
            n = _ln(x_s[j * SP:(j + 1) * SP, :].astype(F32))
        hu = _pack(n * ca1)
        h_s[j * (SP // 2):(j + 1) * (SP // 2), :] = hu
        return hu

    def proj_k(j, hu, dep):
        k = _paced_dot(yes0, hu, wqkv_s[:, D:2 * D], _row_blocks(dep), PACE_LO, PACE_HI)
        k_s[j * (SP // 2):(j + 1) * (SP // 2), :] = _pack(k)

    hs = {0: make_h(0, n0)}
    cp_wk.wait()
    cp_x(2).start()
    hs[1] = make_h(1)
    proj_k(0, hs[0], hs[1])
    cp_x(1).wait()
    cp_bsp.start()
    cp_wm0.start()
    cp_wq.start()
    cp_wv.start()
    hs[2] = make_h(2)
    proj_k(1, hs[1], hs[2])
    hs[3] = make_h(3)
    proj_k(2, hs[2], hs[3])
    cp_x(2).wait()
    for r in range(4):
        cp_wm2(r).start()
    hs[4] = make_h(4)
    proj_k(3, hs[3], hs[4])
    hs[5] = make_h(5)
    proj_k(4, hs[4], hs[5])
    hs[6] = make_h(6)
    proj_k(5, hs[5], hs[6])
    cp_wm0.wait()
    cp_wq.wait()
    cp_wv.wait()
    cp_bsp.wait()
    brow_s[...] = jnp.broadcast_to(bsp_s[0:S].reshape(1, S).astype(F32), (8, S))
    hs[7] = make_h(7)
    wqt = pltpu.bitcast(wqkv_s[:, 0:D].T, U32)
    wvt = pltpu.bitcast(wqkv_s[:, 2 * D:3 * D].T, U32)
    wqvt_s[0:D // 2, :] = wqt
    wqvt_s[D // 2:D, :] = wvt
    proj_k(6, hs[6], jnp.concatenate([hs[7], wqt], axis=0))
    sa = _dot(sc, wmod_s[:, 0:D]).astype(BF16)
    k7a = _paced_dot(yes0, hs[7], wqkv_s[:, D:D + D // 2], _row_blocks(wvt), 0.1, 0.98)
    for part, c0 in enumerate((0, 2 * D)):
        bias = _dot(sa, wqkv_s[:, c0:c0 + D])[0:1]
        for t in range(D // 128):
            qvb_s[part * D + t * 128:part * D + (t + 1) * 128, :] = jnp.broadcast_to(
                bias[:, t * 128:(t + 1) * 128], (128, 128)).T
    k7b = _dot(_unpack(hs[7]), wqkv_s[:, D + D // 2:2 * D])
    k_s[7 * (SP // 2):8 * (SP // 2), :] = _pack(jnp.concatenate([k7a, k7b], axis=1))
    chk_s[0:16, :] = jnp.ones((16, TQ), F32)
    chk_s[16:24, :] = jnp.zeros((8, TQ), F32)
    carp_s[...] = jnp.zeros(carp_s.shape, F32)
    cara_s[...] = jnp.zeros(cara_s.shape, F32)
    kb1_s[2 * NC - 2:2 * NC] = jnp.zeros((2, DH * 8, 128), F32)
    qb1_s[:, S - TQ:S] = jnp.zeros((DH * 8, TQ), F32)
    for cp in (cp_wo, cp_win, cp_wout, cp_wsp):
        cp.start()

    def proj_qv_step(r):
        rows = pl.ds(pl.multiple_of(r * (TP // 2), TP // 2), TP // 2)
        cols = pl.ds(pl.multiple_of(r * TP, TP), TP)
        qvt = _dot_nt(_unpack(wqvt_s[...]), _unpack(h_s[rows, :]))
        qvt = qvt + jnp.concatenate([qvb_s[...]] * (TP // 128), axis=1)
        q = (qvt[0:D] * q_scale).astype(BF16)
        qt_s[:, cols] = pltpu.bitcast(q, U32)
        vt_s[:, cols] = _pack(qvt[D:2 * D])
        vmax = jnp.max(jnp.abs(qvt[D:2 * D]).reshape(D // 8, 8, TP), axis=0)
        chk_s[16:24, :] = jnp.maximum(chk_s[16:24, :], vmax)
        q0 = q[0:DH].astype(F32)
        for d in range(DH):
            qb0_s[d * 8:(d + 1) * 8, cols] = jnp.broadcast_to(q0[d:d + 1], (8, TP))
        k = k_s[rows, :]
        for b in range(D // 128):
            kblk = k[:, b * 128:(b + 1) * 128]
            for j in range(8):
                kh_s[b * 8 + j, rows, :] = kblk if j == 0 else pltpu.roll(kblk, 128 - j * DH, 1)
        for t in range(TP // CK):
            ku = k[t * 64 + POS * 8:t * 64 + POS * 8 + 8, 0:128]
            tg = r * (2 * TP // CK) + 2 * t
            for d in range(DH):
                val = _bcast_k(ku, d)
                kb0_s[tg, d * 8:(d + 1) * 8, :] = val[0:8]
                kb0_s[tg + 1, d * 8:(d + 1) * 8, :] = val[8:16]
        mcols = pl.ds(pl.multiple_of((2 + r) * D, D), D)
        mod_s[:, pl.ds(pl.multiple_of(r * D, D), D)] = _rb(_dot(_unpack(sc_s[...]), wmod_s[:, mcols]))[0:8]
        brow = brow_s[0:1, cols]
        for t in range(TP // 128):
            trow = pl.ds(pl.multiple_of(r * TP + t * 128, 128), 128)
            bcol_s[trow, :] = jnp.broadcast_to(brow[:, t * 128:(t + 1) * 128], (128, 128)).T

    def proj_qv(r, carry):
        for n in range(NP2):
            cp_wm2(r * NP2 + n).wait()
        for n in range(NP2):
            proj_qv_step(r * NP2 + n)
        return carry

    lax.fori_loop(0, S // TP // NP2, proj_qv, 0)

    nt_body = HB * NJ * NC

    def vpu_scores(d, t, half, jj):
        c0 = d["q0"] + jj * 128
        m = d["kb"][2 * t + half] * d["qb"][:, c0:c0 + 128]
        return jnp.sum(jnp.sum(m.reshape(DH // 2, 2, 8, 128), axis=0), axis=0)

    def vpu_group(d, t):
        top = jnp.concatenate([d["pc"][(t, 0, jj)] for jj in range(TQ // 128)], axis=1)
        bot = jnp.concatenate([d["pc"][(t, 1, jj)] for jj in range(TQ // 128)], axis=1)
        d["l"] = d["l"] + (top + bot)
        d["grp"][(t, POS)] = jnp.concatenate([top, bot], axis=0)

    def pv_dot(d, t, vt):
        p = jnp.concatenate([d["grp"][(t, r)] for r in range(8)], axis=0)
        d["acc"] = d["acc"] + _dot(_unpack(vt), p.astype(BF16))

    def finish(d):
        l = jnp.sum(d["l"], axis=0, keepdims=True)
        chk_s[0:1, :] = jnp.minimum(chk_s[0:1, :], l)
        chk_s[8:9, :] = jnp.maximum(chk_s[8:9, :], l)
        ot_s[pl.ds(d["o8"], 8), d["q0"]:d["q0"] + TQ] = _pack(d["acc"] * (1.0 / l))

    def carried_unit(h_prev, o8):
        d = dict(r8=pl.multiple_of(h_prev * 8, 8), o8=o8, q0=(NJ - 1) * TQ,
                 kb=kbs[(HB - 1) % 2], qb=qbs[(HB - 1) % 2],
                 acc=cara_s[0:DH, :], l=cara_s[DH:DH + 8, :], grp={}, pc={})
        for r in range(8):
            d["grp"][(NC - 2, r)] = carp_s[16 * r:16 * r + 16, :]
            if r != POS:
                d["grp"][(NC - 1, r)] = carp_s[CK + 16 * r:CK + 16 * r + 16, :]
        return d

    def attn_fast(i, carry):
        zsrc = qt_s[0:8, 0:128]
        yes = [(zsrc & (1 << b)) <= (1 << b) for b in range(4)]
        st = []
        for un in range(HB * NJ):
            h = i * HB + un // NJ
            r8 = pl.multiple_of(h * 8, 8)
            q0 = (un % NJ) * TQ
            st.append(dict(h=h, r8=r8, o8=r8, q0=q0, kb=kbs[(un // NJ) % 2], qb=qbs[(un // NJ) % 2],
                           qt=_unpack(qt_s[pl.ds(r8, 8), q0:q0 + TQ]),
                           acc=jnp.zeros((DH, TQ), F32), l=jnp.zeros((8, TQ), F32),
                           grp={}, pc={}))
        hp = jnp.maximum(i * HB - 1, 0)
        dc = carried_unit(hp, pl.multiple_of(jnp.where(i == 0, H * 8, hp * 8), 8))

        stream, tile_end, vpu_tiles = [], [], [-1]
        tiles = {-2: (dc, NC - 2), -1: (dc, NC - 1)}
        for un, d in enumerate(st):
            for t in range(NC):
                on_vpu = un >= NJ or t not in SKIP
                if on_vpu:
                    vpu_tiles.append(un * NC + t)
                stream += [(d, t, r) for r in reversed(range(8)) if not (on_vpu and r == POS)]
                tile_end.append(len(stream))
                tiles[un * NC + t] = (d, t)
        pv_at = {(tile_end[ti + 1] if ti + 1 >= 0 else 0) + DELTA: ti for ti in range(-2, nt_body - 2)}
        slots, slot_of_pv = [], {}
        for n in range(len(stream)):
            if n in pv_at:
                slot_of_pv[pv_at[n]] = len(slots)
                slots.append(("v", pv_at[n]))
            slots.append(("k", n))
        ties = {}
        prev_end = -1
        for ti in vpu_tiles[:-1]:
            end = CW if ti == -1 else slot_of_pv[ti] - LEAD if ti in slot_of_pv else len(slots) - 1
            span = end - prev_end
            for n in range(8):
                pos = prev_end + 1 + (n * span) // 8 if span < 8 else end - ((7 - n) * span) // 8
                ties.setdefault(slots[pos], []).append(("pc", ti, n % 2, n // 2))
            prev_end = end
        head_at = (0, tile_end[NJ * NC - 1], len(stream))
        qgroups = [(col, b) for col in range(S // 128) for b in range(0, DH, QG)]
        for hh in range(HB):
            lo_g, span_g = head_at[hh] + RELD + 2, head_at[hh + 1] - head_at[hh] - RELD - GE
            kgroups = [(t, b) for b in range(0, DH, 2) for t in range(NC) if hh == 0 or t not in SKIP]
            for n, g in enumerate(kgroups):
                ties.setdefault(("k", lo_g + (n * span_g) // len(kgroups)), []).append(("kb", hh) + g)
            for n, g in enumerate(qgroups):
                ties.setdefault(("k", lo_g + 1 + (n * span_g) // len(qgroups)), []).append(("qb", hh) + g)
        cuts = set(pv_at) | {0, len(stream)}
        cuts |= {a for a in range(1, len(stream)) if stream[a][0] is not stream[a - 1][0]}
        cuts = sorted(cuts)
        hist = {}

        def side_work(tie, n):
            if tie[0] == "pc":
                _, ti, half, jj = tie
                d, t = tiles[ti]
                s = vpu_scores(d, t, half, jj)
                d["pc"][(t, half, jj)] = jnp.exp2(s)
                return s
            hn = jnp.minimum(i * HB + tie[1] + 1, H - 1)
            if tie[0] == "kb":
                _, hh, tt, b = tie
                src = _after(yes[0], kh_s[hn, pl.ds(tt * 64 + POS * 8, 8), :], hist[n - RELD])
                for dd in range(b, b + 2):
                    val = _bcast_k(src, dd)
                    kbs[(hh + 1) % 2][2 * tt, dd * 8:(dd + 1) * 8, :] = val[0:8]
                    val = val[8:16]
                    kbs[(hh + 1) % 2][2 * tt + 1, dd * 8:(dd + 1) * 8, :] = val
                return val
            _, hh, col, b = tie
            src = qt_s[pl.ds(pl.multiple_of(hn * 8, 8), 8), col * 128:(col + 1) * 128]
            qf = _unpack(_after(yes[0], src, hist[n - RELD])).astype(F32)
            for dd in range(b, b + QG):
                val = jnp.broadcast_to(qf[dd:dd + 1, :], (8, 128))
                qbs[(hh + 1) % 2][dd * 8:(dd + 1) * 8, col * 128:(col + 1) * 128] = val
            return val

        def tied(slot, x):
            for tn, tie in enumerate(ties.get(slot, [])):
                x = _after(yes[tn], x, side_work(tie, slot[1]))
            return x

        for lo, hi in zip(cuts[:-1], cuts[1:]):
            d = stream[lo][0]
            parts = [tied(("k", n), kh_s[d["h"], pl.ds(stream[n][1] * 64 + stream[n][2] * 8, 8), :])
                     for n in range(lo, hi)]
            kk = _unpack(jnp.concatenate(parts, axis=0))[:, 0:DH]
            p = jnp.exp2(_dot(kk, d["qt"]))
            d["l"] = d["l"] + jnp.sum(p.reshape(2 * (hi - lo), 8, TQ), axis=0)
            for n in range(lo, hi):
                _, t, r = stream[n]
                d["grp"][(t, r)] = p[16 * (n - lo):16 * (n - lo) + 16]
                hist[n] = p[16 * (n - lo):16 * (n - lo) + 8, 0:128]
            if hi in pv_at:
                ti = pv_at[hi]
                d, t = tiles[ti]
                if ti in vpu_tiles:
                    vpu_group(d, t)
                pv_dot(d, t, tied(("v", ti), vt_s[pl.ds(d["r8"], 8), t * CK:(t + 1) * CK]))
                if t == NC - 1:
                    finish(d)

        d = st[-1]
        vpu_group(d, NC - 2)
        for r in range(8):
            carp_s[16 * r:16 * r + 16, :] = d["grp"][(NC - 2, r)]
            if r != POS:
                carp_s[CK + 16 * r:CK + 16 * r + 16, :] = d["grp"][(NC - 1, r)]
        cara_s[0:DH, :] = d["acc"]
        cara_s[DH:DH + 8, :] = d["l"]
        return carry

    lax.fori_loop(0, H // HB, attn_fast, 0)

    def o_rows(r0):
        return _unpack(ot_s[0:D // 2, pl.ds(r0, SM1)]).astype(F32).T.astype(BF16)

    o0_s[...] = pltpu.bitcast(o_rows(0), U32)

    dl = carried_unit(H - 1, (H - 1) * 8)
    pv_dot(dl, NC - 2, vt_s[(H - 1) * 8:H * 8, (NC - 2) * CK:(NC - 1) * CK])
    for half in range(2):
        for jj in range(TQ // 128):
            dl["pc"][(NC - 1, half, jj)] = jnp.exp2(vpu_scores(dl, NC - 1, half, jj))
    vpu_group(dl, NC - 1)
    pv_dot(dl, NC - 1, vt_s[(H - 1) * 8:H * 8, (NC - 1) * CK:NC * CK])
    finish(dl)

    def attn_exact(u, carry):
        h = u // NJ
        r8 = pl.multiple_of(h * 8, 8)
        q0 = pl.multiple_of((u % NJ) * TQ, TQ)
        qt = _unpack(qt_s[pl.ds(r8, 8), pl.ds(q0, TQ)])

        def pass1(c, m):
            ku = kh_s[h, pl.ds(pl.multiple_of(c * (CK // 2), CK // 2), CK // 2), :]
            s = _dot(_unpack(ku)[:, 0:DH], qt)
            s_s[pl.ds(pl.multiple_of(c * CK, CK), CK), :] = s
            return jnp.maximum(m, jnp.max(s, axis=0, keepdims=True))

        m = lax.fori_loop(0, NC, pass1, jnp.full((1, TQ), -jnp.inf, F32))

        def pass2(c, la):
            l, acc = la
            c0 = pl.multiple_of(c * CK, CK)
            p = jnp.exp2(s_s[pl.ds(c0, CK), :] - m)
            vt = _unpack(vt_s[pl.ds(r8, 8), pl.ds(c0, CK)])
            return l + jnp.sum(p, axis=0, keepdims=True), acc + _dot(vt, p.astype(BF16))

        l, acc = lax.fori_loop(0, NC, pass2, (jnp.zeros((1, TQ), F32), jnp.zeros((DH, TQ), F32)))
        ot_s[pl.ds(r8, 8), pl.ds(q0, TQ)] = _pack(acc / l)
        return carry

    safe = jnp.logical_and(chk_s[0:1, :] >= L_LO, chk_s[8:9, :] <= L_HI)
    safe = jnp.logical_and(safe, jnp.max(chk_s[16:24, :], axis=0, keepdims=True) <= V_HI)

    @pl.when(jnp.max(jnp.where(safe, 0.0, 1.0)) > 0.0)
    def _():
        lax.fori_loop(0, H * NJ, attn_exact, 0)
        o0_s[...] = pltpu.bitcast(o_rows(0), U32)

    cp_wo.wait()
    cp_win.wait()

    def mix1(r, carry):
        ga = mod_s[0:1, 0:D]
        sb = mod_s[0:1, D:2 * D]
        cb1 = _rb(1.0 + mod_s[0:1, 2 * D:3 * D])

        def stage_a(n):
            r0 = pl.multiple_of(r * TM1 + n * SM1, SM1)
            o = _unpack(o0_s[...]) if n == 0 else o_rows(r0)
            x1 = x_s[pl.ds(r0, SM1), :].astype(F32) + ga * _dot(o, wo_s[...])
            x1_s[pl.ds(r0, SM1), :] = x1
            return (_ln(x1) * cb1 + sb).astype(BF16)

        def stage_b(n, h2):
            r0 = pl.multiple_of(r * TM1 + n * SM1, SM1)
            r2 = pl.multiple_of(r * (TM1 // 2) + n * (SM1 // 2), SM1 // 2)
            z2_s[pl.ds(r2, SM1 // 2), :] = _pack(_ln(_gelu(_dot(h2, win_s[:, FH:2 * FH]))))
            z1_s[pl.ds(r0, SM1), :] = _gelu(_dot(h2, win_s[:, 0:FH]))

        ns = TM1 // SM1
        h2 = [stage_a(n) for n in range(ns)]
        for n in range(ns):
            stage_b(n, h2[n])
        nxt = pl.multiple_of(jnp.minimum(r + 1, S // TM1 - 1) * TM1, TM1)
        o0_s[...] = pltpu.bitcast(o_rows(nxt), U32)
        return carry

    lax.fori_loop(0, S // TM1, mix1, 0)

    cp_wout.wait()
    cp_wsp.wait()

    def cp_out(j):
        rows = pl.ds(pl.multiple_of(j * SM2, SM2), SM2)
        return pltpu.make_async_copy(o_s.at[rows, :], out_hbm.at[0, rows, :], sem_out.at[0])

    def mix2(t, carry):
        gb = mod_s[0:1, 3 * D:4 * D]

        def gate(n):
            t0 = pl.multiple_of(t * TM2 + n * SM2, SM2)
            g = _dot(wsp_s[pl.ds(t0, SM2), :], _unpack(z2_s[...]))
            b = bcol_s[pl.ds(t0, SM2), :]
            g = g + jnp.concatenate([b] * (FH // 128), axis=1)
            return (z1_s[pl.ds(t0, SM2), :] * g).astype(BF16)

        def proj_out(n, u):
            t0 = pl.multiple_of(t * TM2 + n * SM2, SM2)
            res = x1_s[pl.ds(t0, SM2), :] + gb * _dot(u, wout_s[...])
            o_s[pl.ds(t0, SM2), :] = res.astype(BF16)

        ns = TM2 // SM2
        u = [gate(0)]
        for n in range(ns):
            if n + 1 < ns:
                u.append(gate(n + 1))
            proj_out(n, u[n])
            cp_out(t * ns + n).start()
        return carry

    nt = S // TM2
    lax.fori_loop(0, nt, mix2, 0)
    pltpu.make_async_copy(o_s, out_hbm.at[0], sem_out.at[0]).wait()


@jax.jit
def pallas_adaLN_cond__softmax_full_mha__mixer_gmlp__prompt_kernel(
    A_x: jax.Array,
    A_wqkv: jax.Array,
    A_wo: jax.Array,
    B_x: jax.Array,
    B_w_in: jax.Array,
    B_w_sp: jax.Array,
    B_b_sp: jax.Array,
    B_w_out: jax.Array,
    c: jax.Array,
    w_mod: jax.Array,
):
    del B_x
    hbm = pl.BlockSpec(memory_space=pl.ANY)
    scratch = [
        pltpu.VMEM((S, D), BF16),
        pltpu.VMEM((D, 3 * D), BF16),
        pltpu.VMEM((D, D), BF16),
        pltpu.VMEM((D, 2 * FH), BF16),
        pltpu.VMEM((S, S), BF16),
        pltpu.VMEM((4 * S,), BF16),
        pltpu.VMEM((FH, D), BF16),
        pltpu.VMEM((8, 1, D), BF16),
        pltpu.VMEM((D, 6 * D), BF16),
        pltpu.VMEM((8, 4 * D), F32),
        pltpu.VMEM((8, D), U32),
        pltpu.VMEM((8, S), F32),
        pltpu.VMEM((2 * D, 128), F32),
        pltpu.VMEM((D, D), U32),
        pltpu.VMEM((S // 2, D), U32),
        pltpu.VMEM((S // 2, D), U32),
        pltpu.VMEM((H, S // 2, 128), U32),
        pltpu.VMEM((D // 2, S), U32),
        pltpu.VMEM((D // 2, S), U32),
        pltpu.VMEM((D // 2 + 8, S), U32),
        pltpu.VMEM((2 * NC, DH * 8, 128), F32),
        pltpu.VMEM((2 * NC, DH * 8, 128), F32),
        pltpu.VMEM((DH * 8, S), F32),
        pltpu.VMEM((DH * 8, S), F32),
        pltpu.VMEM((32, TQ), F32),
        pltpu.VMEM((2 * CK, TQ), F32),
        pltpu.VMEM((32, TQ), F32),
        pltpu.VMEM((S, TQ), F32),
        pltpu.VMEM((SM1 // 2, D), U32),
        pltpu.VMEM((S, D), F32),
        pltpu.VMEM((S, FH), F32),
        pltpu.VMEM((S // 2, FH), U32),
        pltpu.VMEM((S, 128), F32),
        pltpu.VMEM((S, D), BF16),
        pltpu.SemaphoreType.DMA((11,)),
        pltpu.SemaphoreType.DMA((3,)),
        pltpu.SemaphoreType.DMA((4,)),
        pltpu.SemaphoreType.DMA((1,)),
    ]
    return pl.pallas_call(
        _kernel,
        out_shape=jax.ShapeDtypeStruct((1, S, D), BF16),
        in_specs=[hbm] * 9,
        out_specs=hbm,
        scratch_shapes=scratch,
        compiler_params=pltpu.CompilerParams(vmem_limit_bytes=110 * 1024 * 1024),
    )(A_x, A_wqkv, A_wo, B_w_in, B_w_sp, B_b_sp, B_w_out, c, w_mod)
```
